```python
import os as _os
_os.environ.setdefault("JAX_PLATFORMS", "cpu")
import jax
import jax.numpy as jnp

def _softmax(x, axis=-1):
    return jax.nn.softmax(x, axis=axis)
def _gelu(x):
    return jax.nn.gelu(x, approximate=True)
def _silu(x):
    return jax.nn.silu(x)
def _sigmoid(x):
    return jax.nn.sigmoid(x)
def _layernorm(x, axis=-1, eps=1e-5):
    m = jnp.mean(x, axis=axis, keepdims=True)
    v = jnp.var(x, axis=axis, keepdims=True)
    return (x - m) / jnp.sqrt(v + eps)
def _scatter_add(tgt, idx, src, axis=0):
    return tgt.at[idx].add(src)
def _segment_sum(src, seg, n):
    return jax.ops.segment_sum(src, seg, n)
class _Rng:
    def __init__(self, key):
        self._k = key
    def _next(self):
        self._k, sub = jax.random.split(self._k)
        return sub
    def normal(self, shape):
        return jax.random.normal(self._next(), shape, dtype=jnp.bfloat16)
    def randint(self, lo, hi, shape):
        return jax.random.randint(self._next(), shape, lo, hi, dtype=jnp.int32)
    def uniform(self, shape, lo=0.0, hi=1.0):
        return jax.random.uniform(self._next(), shape, jnp.bfloat16, lo, hi)
    def permutation(self, n):
        return jax.random.permutation(self._next(), n)


kernel_name = 'gated_mix__mha_block__ssm_conv_h3__prompt'

def setup_inputs():
    _rng = _Rng(jax.random.key(int.from_bytes(__import__("os").urandom(4), "little")))
    _w = (lambda a: (lambda t: t.astype(jnp.bfloat16) if jnp.issubdtype(t.dtype, jnp.floating) else t)(jnp.asarray(a)))
    def _A_setup():
        B, S, D, H = 1, 2048, 640, 32
        return {
            "x": _w((lambda *s: _rng.normal(s) * 0.05)(B, S, D)),
            "wqkv": _w((lambda *s: _rng.normal(s) * 0.4)(D, 3 * D)),
            "wo": _w((lambda *s: _rng.normal(s) * 0.05)(D, D)),
        }
    _A_in = _A_setup()

    def _B_setup():
        B, S, D = 1, 2048, 640
        ks = 4
        return {
            "q": _w((lambda *s: _rng.normal(s) * 0.05)(B, S, D)),
            "k": _w((lambda *s: _rng.normal(s) * 0.4)(B, S, D)),
            "v": _w((lambda *s: _rng.normal(s) * 0.4)(B, S, D)),
            "shift_k": _w((lambda *s: _rng.normal(s) * 0.4)(D, ks) * 0.5),
            "ssm_k": _w((lambda *s: _rng.normal(s) * 0.4)(D, S) * (1.0 / S ** 0.5)),
            "ssm_D": _w((lambda *s: _rng.normal(s) * 0.4)(D)),
        }
    _B_in = _B_setup()

    return {
        "A_x": _A_in["x"],
        "A_wqkv": _A_in["wqkv"],
        "A_wo": _A_in["wo"],
        "B_q": _B_in["q"],
        "B_k": _B_in["k"],
        "B_v": _B_in["v"],
        "B_shift_k": _B_in["shift_k"],
        "B_ssm_k": _B_in["ssm_k"],
        "B_ssm_D": _B_in["ssm_D"],
        "gate_w": _w((lambda *s: _rng.normal(s) * 0.05)(640) * 16.0),
    }

def reference(A_x, A_wqkv, A_wo, B_q, B_k, B_v, B_shift_k, B_ssm_k, B_ssm_D, gate_w):
    def _A_ref(x, wqkv, wo):
        B, S, D = x.shape
        H = 32
        Dh = D // H
        qkv = (lambda x, *d: x.transpose(*d))((x @ wqkv).reshape(B, S, 3, H, Dh), 2, 0, 3, 1, 4)
        q, k, v = qkv[0], qkv[1], qkv[2]
        scores = jnp.einsum("bhqd,bhkd->bhqk", q, k) * (Dh ** -0.5)
        p = _softmax(scores, axis=-1)
        o = jnp.einsum("bhqk,bhkd->bhqd", p, v)
        return (lambda x, *d: x.transpose(*d))(o, 0, 2, 1, 3).reshape(B, S, D) @ wo

    def _B_ref(q, k, v, shift_k, ssm_k, ssm_D):
        B, S, D = q.shape
        ks = shift_k.shape[-1]
        k_pad = jnp.pad(k, ((0, 0), (ks - 1, 0), (0, 0)))
        k_shift = jnp.zeros_like(k)
        for t in range(ks):
            k_shift = k_shift + k_pad[:, t:t + S, :] * shift_k[:, ks - 1 - t][None, None, :]
        kv = k_shift * v
        L = 2 * S
        kv_pad = jnp.pad(kv, ((0, 0), (0, S), (0, 0)))
        kf_pad = jnp.pad(ssm_k, ((0, 0), (0, S)))
        kv_f = (lambda x, axes=(-2,-1): jnp.fft.rfft2(x.astype(jnp.float32), axes=axes))(kv_pad[:, None, :, :], axes=(1, 2))
        kf_f = (lambda x, axes=(-2,-1): jnp.fft.rfft2(x.astype(jnp.float32), axes=axes))(kf_pad[:, None, :], axes=(1, 2))
        kf_f = (lambda x, *d: x.transpose(*d))(kf_f, 1, 2, 0)
        y_f = kv_f * kf_f[None, :, :, :]
        y = (lambda x, s, axes=(-2,-1): jnp.fft.irfft2(x, s=s, axes=axes).astype(jnp.bfloat16))(y_f, (1, L), axes=(1, 2))[:, 0, :S, :]
        y = y + kv * ssm_D[None, None, :]
        return q * y

    x = A_x
    g = _sigmoid((x * gate_w).sum(-1, keepdims=True))
    a = _A_ref(x, A_wqkv, A_wo)
    b = _B_ref(x, B_k, B_v, B_shift_k, B_ssm_k, B_ssm_D)
    return g * a + (1 - g) * b
```

```python
import math

import jax
import jax.numpy as jnp
import numpy as np
from jax import lax
import jax.experimental.pallas as pl
import jax.experimental.pallas.tpu as pltpu

S, D, H, KS = 2048, 640, 32, 4
DH = D // H
G = D // 128
F32, BF16, U32 = jnp.float32, jnp.bfloat16, jnp.uint32

XC = 512
BQ, BK = 512, 256
NZ, NQ, NK = BQ // 128, S // BQ, S // BK
STEPS = [(a, j) for j in range(NK) for a in range(NQ)]
DV = 24
NM, NL = G, 1
NA = H - NM - NL
NV = 48
VPU_KEYS = [NV if a == NQ - 1 and j < NK - 1 else 32 for a, j in STEPS]
OUT = [128, 256, 256, 256, 256, 256, 256, 256, 128]
L_LO, L_HI = 2.0 ** -30, 2.0 ** 30

ST = 9
FB = 136


def _low(i):
    return 8 * (i + i // 2 * 2)


def _top(i, bank):
    return 32 * i + 16 + 8 * (bank % 2)


EX0 = _low(NK * DH * NV // 8)
HO0 = EX0 + 6 * 16 * ST
WORK_ROWS = HO0 + _low(160) + 32


def _dot(a, b):
    return lax.dot_general(a, b, (((1,), (0,)), ((), ())), preferred_element_type=F32)


def _dot_nt(a, b):
    return lax.dot_general(a, b, (((1,), (1,)), ((), ())), preferred_element_type=F32)


def _aligned(start, align):
    return start if isinstance(start, int) else pl.multiple_of(start, align)


class _Stores:
    def __init__(self):
        self.pending = []

    def add(self, ref, idx, val, delay=3, tag=None):
        self.pending.append([delay, tag, ref, idx, val])

    def _emit(self, ready):
        for item in self.pending:
            if ready(item):
                item[2][item[3] + (slice(None),)] = item[4]
        self.pending = [item for item in self.pending if not ready(item)]

    def tick(self):
        for item in self.pending:
            item[0] -= 1
        self._emit(lambda item: item[0] <= 0)

    def flush(self, tag=None):
        self._emit(lambda item: tag is None or item[1] == tag)


class _SideWork:
    def __init__(self, items, stores, zero):
        self.items, self.stores, self.zero = list(items), stores, zero
        self.total, self.done = sum(item[0] for item in items), 0

    def pin(self, ref, val):
        val = val.astype(BF16) if ref.dtype == BF16 else pltpu.bitcast(val[:8], ref.dtype)
        rows = pl.ds(self.zero + ref.shape[-2] - val.shape[0], val.shape[0])
        ref[(0,) * (len(ref.shape) - 2) + (rows, slice(None))] = val

    def run_to(self, goal, tick=None):
        pinned = []
        while self.items and self.done < goal:
            for ref in self.items[0][1]:
                if tick is not None and not any(ref is other for other in pinned):
                    self.pin(ref, tick)
                    pinned.append(ref)
            cost = next(self.items[0][2], None)
            if cost is None:
                self.items.pop(0)
            else:
                self.done += cost
        self.stores.tick()

    def finish(self):
        self.run_to(math.inf)
        self.stores.flush()


def _twiddle_table():
    phi1 = (0.25 + np.arange(16)[:, None]) / 16.0
    w2 = np.exp(2j * np.pi * np.arange(1, 16)[None, :] * phi1 / 16.0)
    w2 = np.broadcast_to(w2[:, :, None], (16, 15, 8))
    phi2 = ((phi1 + np.arange(16)[None, :]) / 16.0).reshape(16, 2, 1, 8)
    w3 = np.exp(2j * np.pi * np.arange(1, 8).reshape(1, 1, 7, 1) * phi2 / 8.0).reshape(16, 14, 8)
    w = np.concatenate([w2, w3], 1).reshape(16 * 29, 8)
    w = np.concatenate([w.real, w.imag], 1)
    return np.ascontiguousarray(np.broadcast_to(w[:, :, None], (16 * 29, 16, 128)), dtype=np.float32)


def _cmul(a, w):
    return (a[0] * w[0] - a[1] * w[1], a[0] * w[1] + a[1] * w[0])


def _cmul_conj(a, w):
    return (a[0] * w[0] + a[1] * w[1], a[1] * w[0] - a[0] * w[1])


def _crot(a, k, n):
    k %= n
    if k == 0:
        return a
    c, s = math.cos(2 * math.pi * k / n), math.sin(2 * math.pi * k / n)
    if (8 * k) % n == 0 and (4 * k) % n:
        if c * s > 0:
            return ((a[0] - a[1]) * c, (a[0] + a[1]) * c)
        return ((a[0] + a[1]) * c, (a[1] - a[0]) * c)
    return _cmul(a, (c, s))


def _dft(get, idx, sign, cin=0, put=None, cout=0):
    n = len(idx)
    if n == 1:
        a = get(idx[0])
        yield cin
        return [a]
    if n == 2:
        a, b = get(idx[0]), get(idx[1])
        if a[1] is None:
            y = [(a[0] + b[0], b[1]), (a[0] - b[0], -b[1])]
        else:
            y = [(a[0] + b[0], a[1] + b[1]), (a[0] - b[0], a[1] - b[1])]
        yield 2 * cin + 4
        return y
    e = yield from _dft(get, idx[0::2], sign, cin)
    o1 = yield from _dft(get, idx[1::4], sign, cin)
    o3 = yield from _dft(get, idx[3::4], sign, cin)
    y = [None] * n
    for k in range(n // 4):
        a, b = _crot(o1[k], sign * k, n), _crot(o3[k], 3 * sign * k, n)
        p = (a[0] + b[0], a[1] + b[1])
        m = (a[0] - b[0], a[1] - b[1])
        e0, e1 = e[k], e[k + n // 4]
        y[k] = (e0[0] + p[0], e0[1] + p[1])
        y[k + n // 2] = (e0[0] - p[0], e0[1] - p[1])
        up = (e1[0] - m[1], e1[1] + m[0])
        dn = (e1[0] + m[1], e1[1] - m[0])
        y[k + n // 4], y[k + 3 * n // 4] = (up, dn) if sign > 0 else (dn, up)
        if put is not None:
            for j in range(k, n, n // 4):
                put(j, y[j])
        yield 12 + (0 if k == 0 else 8 if 8 * k == n else 12) + 4 * cout
    return y


def _fft_first(src, dst, st, g, row):
    def get(n):
        a = src[g, pl.ds(FB * n + row, 8), :]
        return (a * math.cos(math.pi * n / 32), a * math.sin(math.pi * n / 32)) if n else (a, None)

    def put(j, y):
        for z in range(2):
            st.add(dst, (z, g, pl.ds(FB * j + row, 8)), y[z])
    return 200, (src, dst), _dft(get, list(range(16)), 1, 2, put)


def _fft_middle(fu, fh, work, st, tw, g, b):
    twiddle = lambda i: (tw[b * 29 + i, 0:8], tw[b * 29 + i, 8:16])
    w2 = lambda n: twiddle(n - 1)
    w3 = lambda half, n: twiddle(14 + 7 * half + n)
    p2w = 6

    def save(area, exchange):
        def put(i, y):
            for z in range(2):
                row = EX0 + ((2 * area + z) * 16 + i) * ST if exchange else HO0 + _low(32 * area + 2 * i + z)
                st.add(work, (pl.ds(row, 8),), y[z], tag=(area, exchange))
        return put

    def saved(area, i):
        return tuple(work[pl.ds(HO0 + _low(32 * area + 2 * i + z), 8), :] for z in range(2))

    def exchanged(area, i):
        return tuple(work[pl.ds(EX0 + ((2 * area + z) * 16 + i // 8 * 8) * ST + i % 8, 8, stride=ST), :]
                     for z in range(2))

    def pass1(area, get, sign, cin):
        st.flush((area, True))
        for m in range(4):
            put = lambda k, y: save(area, False)(4 * m + k, y if (m * k) % 4 == 0 else _crot(y, sign * m * k, 16))
            yield from _dft(get, list(range(m, 16, 4)), sign, cin, put, (0, 4, 2, 4)[m])

    def pass2(area, put, sign, cout):
        st.flush((area, False))
        for k in range(4):
            x = [saved(area, 4 * m + k) for m in range(4)]
            if k == 2:
                e = [(x[0][0] - x[2][1], x[0][1] + x[2][0]), (x[0][0] + x[2][1], x[0][1] - x[2][0])][::sign]
            else:
                e = [(x[0][0] + x[2][0], x[0][1] + x[2][1]), (x[0][0] - x[2][0], x[0][1] - x[2][1])]
            p = (x[1][0] + x[3][0], x[1][1] + x[3][1])
            q = (x[1][0] - x[3][0], x[1][1] - x[3][1])
            put(k, (e[0][0] + p[0], e[0][1] + p[1]))
            put(k + 8, (e[0][0] - p[0], e[0][1] - p[1]))
            yield 10 + 2 * cout + p2w
            put(k + 8 - 4 * sign, (e[1][0] - q[1], e[1][1] + q[0]))
            put(k + 8 + 4 * sign, (e[1][0] + q[1], e[1][1] - q[0]))
            yield 6 + 2 * cout + p2w

    def residue(src):
        def get(n):
            a = tuple(src[z, g, pl.ds(b * FB + 8 * n, 8), :] for z in range(2))
            return _cmul(a, w2(n)) if n else a
        return get

    def spectrum(s, half):
        st.flush((s, True))
        get = lambda n: _cmul(exchanged(s, 8 * half + n), w3(half, n)) if n else exchanged(s, 8 * half)
        yield from _dft(get, list(range(8)), 1, 6, lambda j, y: save(3 + half, False)(8 * s + j, y))

    def product(half):
        st.flush((3 + half, False))
        put = lambda n, y: save(2, True)(8 * half + n, _cmul_conj(y, w3(half, n)) if n else y)
        yield from _dft(lambda j: _cmul(saved(3 + half, j), saved(3 + half, 8 + j)), list(range(8)), -1, 6, put, 6)

    def result(n, y):
        a = _cmul_conj(y, w2(n)) if n else y
        for z in range(2):
            st.add(fu, (z, g, pl.ds(b * FB + 8 * n, 8)), a[z])

    forward = [(200, (fu,), pass1(0, residue(fu), 1, 6)), (200, (fh,), pass1(1, residue(fh), 1, 6))]
    forward += [(64 + 8 * p2w, (), pass2(s, save(s, True), 1, 0)) for s in range(2)]
    forward += [(104, (), spectrum(s, half)) for s in range(2) for half in range(2)]
    forward += [(152, (), product(half)) for half in range(2)]
    return forward, [(104, (), pass1(2, lambda j: exchanged(2, j), -1, 0)),
                     (160 + 8 * p2w, (fu,), pass2(2, result, -1, 6))]


def _fft_last(src, dst, st, g, row):
    def put(n, y):
        a = y[0] * (math.cos(math.pi * n / 32) / S)
        st.add(dst, (g, pl.ds(FB * n + row, 8)), a + y[1] * (math.sin(math.pi * n / 32) / S) if n else a)
    get = lambda j: tuple(src[z, g, pl.ds(FB * j + row, 8), :] for z in range(2))
    return 216, (src, dst), _dft(get, list(range(16)), -1, 0, put, 3)


def _kernel(x_hbm, wqkv_hbm, wo_hbm, k_hbm, v_hbm, ssm_hbm, tw_hbm, shift_hbm, dvec_hbm, gate_hbm, out_hbm,
            x_v, w_v, wo_v, k_v, v_v, ssm_v, tw_v, out_v, kg, qh, vt, ot, u_s, h_s, fu, fh, k32, q32,
            work, pb0, pb1, qw, kf, o_first, wt, gate_s, shift_v, dvec_v, gate_v, zero_s, sems, osems):
    st = _Stores()
    slow = 7
    lead = 200
    runtime_zero = lambda i: pl.multiple_of(16 * (i >> 6), 16)

    copies = []

    def copy(src, dst):
        copies.append(pltpu.make_async_copy(src, dst, sems.at[len(copies)]))
        return copies[-1]

    rows_copy = lambda src, dst, start, size: copy(src.at[pl.ds(start, size)], dst.at[pl.ds(start, size)])
    cp_x = [rows_copy(x_hbm, x_v, r, XC) for r in range(0, S, XC)]
    cp_w = [copy(wqkv_hbm.at[:, pl.ds(i * D, D)], w_v.at[i]) for i in range(3)]
    cp_k = [rows_copy(k_hbm, k_v, r, S // 2) for r in (0, S // 2)]
    cp_v = [rows_copy(v_hbm, v_v, r, S // 2) for r in (0, S // 2)]
    cp_ssm = [rows_copy(ssm_hbm, ssm_v, 0, D - 128), rows_copy(ssm_hbm, ssm_v, D - 128, 128)]
    cp_tw = copy(tw_hbm, tw_v.at[:, pl.ds(0, 16)])
    cp_wo = copy(wo_hbm, wo_v)
    cp_small = [copy(shift_hbm, shift_v.at[:, pl.ds(0, D)]), copy(dvec_hbm, dvec_v), copy(gate_hbm, gate_v)]

    def start(*cps):
        for cp in cps:
            cp.start()

    def wait(*cps):
        for cp in cps:
            cp.wait()

    start(cp_w[1], cp_x[0], *cp_small)

    def clear(i, _):
        row = pl.multiple_of(_top(i, 0), 16)
        pb1.bitcast(U32)[pl.ds(row, 16), :] = jnp.zeros((16, 128), U32)
        for half in range(2):
            qw[pl.ds(row + 32 * 64 * half, 16), :] = jnp.zeros((16, 128), U32)
        zero_s[0] = i >> 6
    lax.fori_loop(0, 64, clear, None)
    ot[0, :, pl.ds(S - BQ, BQ)] = jnp.zeros((DV, BQ), F32)

    def weight_block(n, i, j):
        st.add(wt, (n, j, pl.ds(128 * i, 128)), w_v[2 * n, pl.ds(128 * j, 128), pl.ds(128 * i, 128)].T, slow)
        yield 40

    def gate_block(r):
        xf = x_v[pl.ds(r, 64), :].astype(F32)
        logit = jnp.sum(xf * gate_v[...].astype(F32).reshape(1, D), axis=-1, keepdims=True)
        st.add(gate_s, (pl.ds(r, 64),), jnp.broadcast_to(jax.nn.sigmoid(logit), (64, 128)), slow)
        yield 200

    weights = lambda n: [(40, (wt,)[n:], weight_block(n, i, j)) for i in range(G) for j in range(G)]
    gates = lambda c: [(200, (gate_s,), gate_block(r)) for r in range(c * XC, c * XC + XC, 64)]
    last_group = lambda h: (DH * h + DH - 1) >> 7

    def key_group(h):
        first = (DH * h) >> 7
        return first + G * (last_group(h) - first)

    def project_k(r0, n, items):
        rest = [_dot(x_v[pl.ds(r0 + i * n // 4, n // 4), 512:], w_v[1, 512:, 512:]) for i in range(4)]
        rest = jnp.concatenate([_dot(x_v[pl.ds(r0, n), 512:], w_v[1, 512:, :512]), jnp.concatenate(rest, 0)], 1)
        groups = [_dot(x_v[pl.ds(r0, n), :512], w_v[1, :512, 128 * g:128 * g + 128]) + rest[:, 128 * g:128 * g + 128]
                  for g in range(G)]
        groups = [val * (DH ** -0.5 * math.log2(math.e)) for val in groups]
        left = lax.broadcasted_iota(jnp.int32, (n, 128), 1) < 64
        groups += [jnp.where(left, groups[g + 1], groups[g]) for g in range(G - 1)]
        for g in (0, 1, 5, 2, 6, 3, 7, 4, 8):
            for r in range(n // 16):
                kg[g, pl.ds(2 * _low(r0 // 16 + r), 16), :] = groups[g][16 * r:16 * r + 16].astype(BF16)
        side = _SideWork(items, st, runtime_zero(zero_s[0]))
        for g in range(G + 1):
            ready = [(h, j) for j in range(n // BK) for h in range(NA) if last_group(h) == g - 1]
            for i in range(8):
                for h, j in ready[i * len(ready) // 8:(i + 1) * len(ready) // 8]:
                    val = groups[key_group(h)][BK * (j + 1) - NV:BK * (j + 1)]
                    k32[h, r0 // BK + j, :NV] = pltpu.roll(val, -DH * h % 128, 1) if h and g < G else val
                if g < G:
                    tick = groups[g][i * n // 8:i * n // 8 + 16]
                    side.pin(k32, tick)
                    side.run_to(side.total * (8 * g + i + 1) / 33, tick)
        side.finish()

    wait(*cp_small, cp_w[1])
    start(cp_x[1], cp_x[2])
    wait(cp_x[0])
    project_k(0, XC, gates(0))
    start(cp_x[3], cp_w[0])
    wait(cp_x[1])
    project_k(XC, XC, gates(1))
    wait(cp_x[2], cp_x[3])
    start(cp_ssm[0], cp_k[0])
    wait(cp_w[0])
    items = weights(0)
    for i, item in enumerate(gates(2)):
        items.insert(4 * i, item)
    project_k(2 * XC, 2 * XC, items)

    def project_t(n, chunks, emit, items):
        side = _SideWork(items, st, runtime_zero(zero_s[0]))
        side.run_to(lead)
        weight = lambda j: pltpu.bitcast(wt.bitcast(U32)[n, j, :D // 2], BF16)
        ticks, count = len(chunks) * (XC // 128 + 1) * (D // 32), 0

        def pace(val):
            nonlocal count
            for r in range(0, D, 32):
                count += 1
                side.run_to(lead + (side.total - lead) * 1.02 * count / ticks, val[r:r + 16, 0:128])

        for c in chunks:
            rest = _dot_nt(weight(G - 1), x_v[pl.ds(c * XC, XC), 512:])
            pace(rest)
            for z in range(XC // 128):
                val = _dot_nt(jnp.concatenate([weight(j) for j in range(G - 1)], 1),
                              x_v[pl.ds(c * XC + 128 * z, 128), :512]) + rest[:, 128 * z:128 * z + 128]
                emit(c * XC // 128 + z, val)
                pace(val)
        side.finish()

    sub = lax.broadcasted_iota(jnp.int32, (8, 128), 0)

    def emit_q(z, val):
        q32[pl.ds(z * D, NA * DH), :] = val[:NA * DH]
        for h in range(H):
            lo, hi = DH * h, DH * (h + 1)
            parts = []
            for r in range(lo // 16 * 16, lo // 16 * 16 + 32, 8):
                part = val[r:r + 8]
                parts.append(jnp.zeros((8, 128), F32) if r + 8 <= lo or r >= hi else
                             jnp.where(sub >= lo - r, part, 0.0) if r < lo else
                             jnp.where(sub < hi - r, part, 0.0) if r + 8 > hi else part)
            qh[h, pl.ds(32 * z, 32), :] = jnp.concatenate(parts, 0).astype(BF16)

    def emit_v(z, val):
        for h in range(0, H, 2):
            r = DH * h
            mid = val[r + 16:r + 24]
            vt[h, pl.ds(32 * z, DV), :] = jnp.concatenate([val[r:r + 16], jnp.where(sub < 4, mid, 1.0)], 0)
            vt[h + 1, pl.ds(32 * z, DV), :] = jnp.concatenate([jnp.where(sub < 4, 1.0, mid), val[r + 24:r + 40]], 0)

    def filter_block(g, z):
        st.add(h_s, (g, pl.ds(z * FB, 128)), ssm_v[pl.ds(128 * g, 128), pl.ds(128 * z, 128)].astype(F32).T, slow)
        yield 40

    def signal_block(g, z):
        cols = pl.ds(128 * g, 128)
        w = shift_v[:, cols].astype(F32)
        base = z % 2 * FB
        stage = kf.at[pl.ds(runtime_zero(zero_s[0]), 2 * FB)]
        stage[pl.ds(base, 8), :] = k_v[pl.ds(128 * z - 16, 16), cols].astype(F32)[8:] if z else jnp.zeros((8, 128), F32)
        stage[pl.ds(base + 8, 128), :] = k_v[pl.ds(128 * z, 128), cols].astype(F32)
        yield 40
        for r in range(0, 128, 32):
            acc = kf[pl.ds(base + 8 + r, 32), :] * w[0:1]
            for t in range(1, KS):
                acc = acc + kf[pl.ds(base + 8 + r - t, 32), :] * w[t:t + 1]
            st.add(u_s, (g, pl.ds(z * FB + r, 32)), acc * v_v[pl.ds(128 * z + r, 32), cols].astype(F32))
            yield 44

    def stores_done():
        st.flush()
        yield 0

    filters = lambda g: [(40, (h_s,), filter_block(g, z)) for z in range(16)]
    signals = lambda i: [(216, (kf, u_s), signal_block(g, z)) for g in range(G) for z in range(8 * i, 8 * i + 8)]
    first = lambda src, dst, g: [(0, (), stores_done())] + [_fft_first(src, dst, st, g, r) for r in range(0, 128, 8)]

    start(cp_v[0], cp_w[2], cp_ssm[1])
    wait(cp_ssm[0])
    items = filters(0)
    for i, item in enumerate(gates(3)):
        items.insert(3 * i, item)
    for g in range(3):
        passes = first(h_s, fh, g)
        for i, item in enumerate(filters(g + 1)):
            passes.insert(1 + i + i * 3 // 4, item)
        items += passes
    project_t(0, (0, 1), emit_q, items)
    start(cp_k[1], cp_v[1])
    wait(cp_k[0], cp_v[0], cp_w[2], cp_ssm[1])
    items = filters(4)
    project_t(0, (2, 3), emit_q, first(h_s, fh, 3) + items[:1]
              + [item for pair in zip(signals(0), weights(1) + items[1:], strict=True) for item in pair])

    kg32, qh32 = kg.bitcast(U32), qh.bitcast(U32)
    kb_row = lambda j, i, d: _low(((j * (NV // 16) + i // 2) * DH + d) * 2 + i % 2)
    qb_row = lambda z, d: _top(z // 2 * DH + d, z)
    p_row = lambda r, z: 2 * _top(r * NZ + z, z + min(r // 8, 1))

    def spread_keys(h, j, d, nv):
        col = jnp.broadcast_to(k32[h, j, NV - nv:NV, d:d + 1], (nv, 128))
        for i in range(nv // 8):
            work[pl.ds(kb_row(j, (NV - nv) // 8 + i, d), 8), :] = col[8 * i:8 * i + 8]

    def spread_query(h, z, d):
        work[pl.ds(qb_row(z, d), 8), :] = jnp.broadcast_to(q32[pl.ds(z * D + DH * h + d, 1), :], (8, 128))

    def stage_queries(h, z):
        slot = lambda r: pl.ds(pl.multiple_of(_top(8 * z + (r & 7), z), 8), 8)
        for i in range(2):
            qw[slot(((DH * jnp.maximum(h - 1, 0)) >> 4) + i), :] = jnp.zeros((8, 128), U32)
        for i in range(2):
            qw[slot(((DH * h) >> 4) + i), :] = qh32[h, pl.ds(16 * z + 8 * i, 8), :]

    def query_tiles(z0, n):
        tiles = [jnp.concatenate([qw[pl.ds(_top(8 * z + r, z), 8), :] for r in range(8)], 0) for z in range(z0, z0 + n)]
        return pltpu.bitcast(jnp.concatenate(tiles, 1), BF16)

    def key_rows(grp, r0, n):
        return pltpu.bitcast(jnp.concatenate([kg32[grp, pl.ds(_low(r), 8), :] for r in range(r0, r0 + n)], 0), BF16)

    def value_tiles(h, k0, n):
        return jnp.concatenate([vt[h, pl.ds(32 * k, DV), :] for k in range(k0, k0 + n)], 1)

    def late_keys():
        for h in range(NA):
            if last_group(h) == G - 1:
                for j in range(NK):
                    k32[h, j, :NV] = pltpu.roll(k32[h, j, :NV], -DH * h % 128, 1)
                    yield 10

    def first_operands():
        for d in range(DH):
            spread_keys(0, 0, d, NV)
            yield 20
        for z in range((NQ - 1) * NZ):
            stage_queries(0, z)
        for z in range(2 * NZ):
            for d in range(DH):
                spread_query(0, z, d)
            yield 40

    start(cp_tw, cp_wo)
    wait(cp_k[1], cp_v[1])
    project_t(1, (0, 1, 2, 3), emit_v,
              [(80, (), late_keys())] + first(h_s, fh, 4) + [(720, (work,), first_operands())] + signals(1)
              + [item for g in range(G) for item in first(u_s, fu, g)])
    wait(cp_tw)

    def vpu_scores(a, j, pair, z0, slot, p_out):
        acc = [None, None]
        for d in range(DH):
            keys = jnp.concatenate([work[pl.ds(kb_row(j, 2 * pair + i, d), 8), :] for i in range(2)], 0)
            for i in range(2):
                qrow = work[pl.ds(qb_row(a * NZ + z0 + i, d), 8), :]
                term = keys * jnp.concatenate([qrow, qrow], 0)
                acc[i] = acc[i] + term if d else term
            if d == DH - 1:
                for i in range(2):
                    p_out[pl.ds(p_row(slot, z0 + i), 16), :] = jnp.exp2(acc[i]).astype(BF16)
            yield

    def weighted_values(h, t, nv):
        src = (pb0, pb1)[t % 2].bitcast(U32)
        slots = [BK // 16 if nv == NV and r == (BK - NV) // 16 else r for r in range(BK // 16)]
        p = [jnp.concatenate([src[pl.ds(p_row(r, z) // 2, 8), :] for r in slots], 0) for z in range(NZ)]
        return _dot(value_tiles(h, STEPS[t][1] * BK // 128, BK // 128), pltpu.bitcast(jnp.concatenate(p, 1), BF16))

    def head(h, items):
        is_last, shared = isinstance(h, int), not items
        side = _SideWork(items, st, runtime_zero(zero_s[0] if is_last else h))
        grp, nxt = key_group(h), jnp.minimum(h + 1, NA - 1)
        nvs = VPU_KEYS if shared else [0] * len(STEPS)
        pv_span = 52 if shared else 36
        p_outs = [pb.at[pl.ds(side.zero, pb.shape[0] - 64)] for pb in (pb0, pb1)]
        blocks, due = [], []
        for t, (a, j) in enumerate(STEPS):
            if shared:
                blocks += [(a, j, pair, z0, (BK - NV) // 16 + pair, p_outs[t % 2]) for pair in (1, 2) for z0 in (0, 2)]
            due.append(DH * len(blocks))
            if a % 2 == 0 and nvs[NQ * j + NQ - 1] == NV:
                blocks.append((NQ - 1, j, 0, a, BK // 16, p_outs[1]))
                due[-1] += DH // 2
        scores, scored = (None for block in blocks for _ in vpu_scores(*block)), 0
        side.run_to(lead)
        if shared:
            for z in range(2 * NZ, NQ * NZ):
                for d in range(DH):
                    spread_query(h, z, d)
        acc, res = {}, None
        for t, (a, j) in enumerate(STEPS):
            rows = BK - nvs[t]
            s = _dot(key_rows(grp, j * BK // 16, rows // 16), query_tiles(a * NZ, NZ))
            if t:
                side.pin(qw, res[0:8, 0:128])
            if t == 0 or (t > len(STEPS) - NQ and not is_last):
                for z in range(NZ):
                    stage_queries(h + 1 if t else h, (a - 1) % NQ * NZ + z)

            def advance(tick, clock, begin=scored):
                nonlocal scored
                frac = clock / (rows + pv_span)
                while scored < begin + (due[t] - begin) * frac - 1e-6:
                    next(scores)
                    scored += 1
                side.run_to(lead + (side.total - lead) * (t + frac) / len(STEPS), tick)

            for r in range(rows // 16):
                for z in range(NZ):
                    p_outs[t % 2][pl.ds(p_row(r, z), 16), :] = jnp.exp2(
                        s[16 * r:16 * r + 16, 128 * z:128 * z + 128]).astype(BF16)
                tick = s[16 * r:16 * r + 8, 0:128]
                side.pin(work, tick)
                if shared and r % 3 == 0:
                    jn = (j + 1) % NK
                    spread_keys(h if jn else nxt, jn, a * DH // NQ + r // 3, max(nvs[NQ * jn:NQ * jn + NQ]))
                if shared and t >= len(STEPS) - 2 and r < 12:
                    for i in range(r * NZ * DH // 12, (r + 1) * NZ * DH // 12):
                        spread_query(nxt, (t - len(STEPS) + 2) * NZ + i // DH, i % DH)
                advance(tick, 16 * (r + 1))
            if t == 0:
                res = weighted_values(jnp.maximum(h - 1, 0), len(STEPS) - 1, 0)
                ot[h, :, pl.ds(S - BQ, BQ)] += res
            else:
                a, j = STEPS[t - 1]
                res = weighted_values(h, t - 1, nvs[t - 1])
                acc[a] = acc[a] + res if j else res
                if t + NQ >= len(STEPS):
                    ot[h + 1, :, pl.ds(a * BQ, BQ)] = acc[a]
            for i, tick in enumerate((res[0:8, 0:128], res[16:24, 0:128], res[8:16, 256:384])):
                side.pin(work, tick)
                advance(tick, rows + pv_span * (i + 1) / 3)
            assert scored == due[t]
        side.finish()

    def middle(g):
        items, back = [], []
        for b in range(16):
            forward, inverse = _fft_middle(fu, fh, work, st, tw_v, g, b)
            items += forward[:1] + back[:1] + forward[1:2] + back[1:] + forward[2:]
            back = inverse
        return items + back

    lax.fori_loop(0, NA, lambda h, _: head(h, []), None)
    lax.fori_loop(0, NM, lambda g, _: head(NA + g, middle(g)), None)
    head(H - 1, [_fft_last(fu, h_s, st, g, r) for g in range(G) for r in range(0, 128, 8)])

    def normalize(z):
        cols = pl.ds(_aligned(z * 128, 128), 128)
        parts, lo, hi = [], None, None
        for h in range(0, H, 2):
            even, odd = ot[h + 1, :, cols], ot[h + 2, :, cols]
            denom = jnp.where(sub < 4, odd[0:8], even[16:24])
            lo, hi = (jnp.minimum(lo, denom), jnp.maximum(hi, denom)) if h else (denom, denom)
            inv = 1.0 / denom
            ie, io = inv[4:5], inv[0:1]
            parts += [even[0:16] * ie, jnp.where(sub < 4, even[16:24] * ie, odd[0:8] * io), odd[8:24] * io]
        return jnp.concatenate(parts, 0).T.astype(BF16), jnp.where((lo >= L_LO) & (hi <= L_HI), 0.0, 1.0)

    def mix(z0, o):
        n = o.shape[0]
        rows = pl.ds(_aligned(z0 * 128, 128), n)
        a = _dot(o, wo_v[...])
        gate = jnp.concatenate([gate_s[rows, :]] * G, 1)
        plane = lambda ref: jnp.concatenate([jnp.concatenate(
            [ref[g, pl.ds(_aligned((z0 + z) * FB, 8), 128), :] for z in range(n // 128)], 0) for g in range(G)], 1)
        b = x_v[rows, :].astype(F32) * (plane(h_s) + plane(u_s) * dvec_v[...].astype(F32).reshape(1, D))
        out_v[rows, :] = (gate * a + (1.0 - gate) * b).astype(BF16)

    def out_copy(r0, n, sem):
        return pltpu.make_async_copy(out_v.at[pl.ds(r0, n)], out_hbm.at[pl.ds(r0, n)], osems.at[sem])

    o_first[...], unsafe = normalize(0)
    wait(cp_wo)
    ot[H, :, pl.ds(S - BQ, BQ)] += weighted_values(H - 1, len(STEPS) - 1, 0)
    cp_out = [out_copy(sum(OUT[:i]), n, i) for i, n in enumerate(OUT)]
    for i, n in enumerate(OUT):
        z = sum(OUT[:i]) // 128
        if i:
            o, flags = zip(*[normalize(z + e) for e in range(n // 128)])
            unsafe = unsafe + sum(flags)
        mix(z, jnp.concatenate(o, 0) if i else o_first[...])
        cp_out[i].start()
    unsafe = jnp.max(unsafe)
    wait(*cp_out)

    @pl.when(unsafe > 0.0)
    def _():
        def attend(i, _):
            h, z = i // (S // 128), i % (S // 128)
            for r in range(8):
                qw[pl.ds(_top(r, 0), 8), :] = jnp.zeros((8, 128), U32)
            for r in range(2):
                qw[pl.ds(pl.multiple_of(_top((((DH * h) >> 4) + r) & 7, 0), 8), 8), :] = (
                    qh32[h, pl.ds(pl.multiple_of(16 * z + 8 * r, 8), 8), :])
            s = _dot(key_rows(key_group(h), 0, S // 16), query_tiles(0, 1))
            p = jnp.exp2(s - jnp.max(s, axis=0, keepdims=True)).astype(BF16)
            ot[h + 1, :, pl.ds(pl.multiple_of(z * 128, 128), 128)] = _dot(value_tiles(h, 0, S // 128), p)
        lax.fori_loop(0, H * (S // 128), attend, None)
        lax.fori_loop(0, S // 128, lambda z, _: mix(z, normalize(z)[0]), None)
        whole = out_copy(0, S, 0)
        whole.start()
        whole.wait()


@jax.jit
def pallas_gated_mix__mha_block__ssm_conv_h3__prompt_kernel(
    A_x: jax.Array,
    A_wqkv: jax.Array,
    A_wo: jax.Array,
    B_q: jax.Array,
    B_k: jax.Array,
    B_v: jax.Array,
    B_shift_k: jax.Array,
    B_ssm_k: jax.Array,
    B_ssm_D: jax.Array,
    gate_w: jax.Array,
):
    del B_q
    tw = _twiddle_table()
    hbm = pl.BlockSpec(memory_space=pl.ANY)
    vmem = pltpu.VMEM
    out = pl.pallas_call(
        _kernel,
        in_specs=[hbm] * 10,
        out_specs=hbm,
        out_shape=jax.ShapeDtypeStruct((S, D), BF16),
        scratch_shapes=[
            vmem((S, D), BF16), vmem((3, D, D), BF16), vmem((D, D), BF16),
            vmem((S, D), BF16), vmem((S, D), BF16), vmem((D, S), BF16),
            vmem((tw.shape[0], 32, 128), F32), vmem((S, D), BF16),
            vmem((2 * G - 1, 2 * _low(S // 16), 128), BF16),
            vmem((H, S // 4, 128), BF16), vmem((H, S // 4, 128), F32),
            vmem((H + 1, DV, S), F32),
            vmem((G, 16 * FB, 128), F32), vmem((G, 16 * FB, 128), F32),
            vmem((2, G, 16 * FB, 128), F32), vmem((2, G, 16 * FB, 128), F32),
            vmem((NA, NK, NV + 16, 128), F32), vmem((S // 128 * D, 128), F32),
            vmem((WORK_ROWS, 128), F32),
            vmem((4 * NZ * (BK + 16) + 64, 128), BF16),
            vmem((4 * NZ * (BK + 16) + 64, 128), BF16),
            vmem((2 * S + 32, 128), U32), vmem((2 * FB + 16, 128), F32),
            vmem((128, D), BF16), vmem((2, G, D + 64, 128), BF16),
            vmem((S + 32, 128), F32),
            vmem((KS, 1536), BF16), vmem((D,), BF16), vmem((D,), BF16),
            pltpu.SMEM((1,), jnp.int32),
            pltpu.SemaphoreType.DMA((18,)), pltpu.SemaphoreType.DMA((len(OUT),)),
        ],
        compiler_params=pltpu.CompilerParams(vmem_limit_bytes=124 * 2 ** 20),
    )(A_x.reshape(S, D), A_wqkv, A_wo, B_k.reshape(S, D), B_v.reshape(S, D), B_ssm_k, tw,
      B_shift_k.T, B_ssm_D, gate_w)
    return out.reshape(1, S, D)
```

```python
import math

import jax
import jax.numpy as jnp
import numpy as np
from jax import lax
import jax.experimental.pallas as pl
import jax.experimental.pallas.tpu as pltpu

S, D, H, KS = 2048, 640, 32, 4
DH = D // H
G = D // 128
F32, BF16, U32 = jnp.float32, jnp.bfloat16, jnp.uint32

XC = 512
BQ, BK = 512, 256
NZ, NQ, NK = BQ // 128, S // BQ, S // BK
STEPS = [(a, j) for j in range(NK) for a in range(NQ)]
DV = 24
NM, NL = G, 1
NA = H - NM - NL
NV = 48
VPU_KEYS = [NV if a == NQ - 1 and j < NK - 1 else 32 for a, j in STEPS]
OUT = [128, 256, 256, 256, 256, 256, 256, 256, 128]
KROWS = [256, 512, 768, 512]
L_LO, L_HI = 2.0 ** -30, 2.0 ** 30

ST = 9
FB = 136


def _low(i):
    return 8 * (i + i // 2 * 2)


def _top(i, bank):
    return 32 * i + 16 + 8 * (bank % 2)


EX0 = _low(NK * DH * NV // 8)
HO0 = EX0 + 6 * 16 * ST
WORK_ROWS = HO0 + _low(128) + 32


def _dot(a, b):
    return lax.dot_general(a, b, (((1,), (0,)), ((), ())), preferred_element_type=F32)


def _dot_nt(a, b):
    return lax.dot_general(a, b, (((1,), (1,)), ((), ())), preferred_element_type=F32)


def _aligned(start, align):
    return start if isinstance(start, int) else pl.multiple_of(start, align)


class _Stores:
    def __init__(self):
        self.pending = []

    def add(self, ref, idx, val, delay=3, tag=None):
        self.pending.append([delay, tag, ref, idx, val])

    def _emit(self, ready):
        for item in self.pending:
            if ready(item):
                item[2][item[3] + (slice(None),)] = item[4]
        self.pending = [item for item in self.pending if not ready(item)]

    def tick(self):
        for item in self.pending:
            item[0] -= 1
        self._emit(lambda item: item[0] <= 0)

    def flush(self, tag=None):
        self._emit(lambda item: tag is None or item[1] == tag)


class _SideWork:
    def __init__(self, items, stores, zero):
        self.items, self.stores, self.zero = list(items), stores, zero
        self.total, self.done = sum(item[0] for item in items), 0

    def pin(self, ref, val):
        val = val.astype(BF16) if ref.dtype == BF16 else pltpu.bitcast(val[:8], ref.dtype)
        rows = pl.ds(self.zero + ref.shape[-2] - val.shape[0], val.shape[0])
        ref[(0,) * (len(ref.shape) - 2) + (rows, slice(None))] = val

    def run_to(self, goal, tick=None):
        pinned = []
        while self.items and self.done < goal:
            for ref in self.items[0][1]:
                if tick is not None and not any(ref is other for other in pinned):
                    self.pin(ref, tick)
                    pinned.append(ref)
            cost = next(self.items[0][2], None)
            if cost is None:
                self.items.pop(0)
            else:
                self.done += cost
        self.stores.tick()

    def finish(self):
        self.run_to(math.inf)
        self.stores.flush()


def _twiddle_table():
    phi1 = (0.25 + np.arange(16)[:, None]) / 16.0
    w2 = np.exp(2j * np.pi * np.arange(1, 16)[None, :] * phi1 / 16.0)
    w2 = np.broadcast_to(w2[:, :, None], (16, 15, 8))
    phi2 = ((phi1 + np.arange(16)[None, :]) / 16.0).reshape(16, 2, 1, 8)
    w3 = np.exp(2j * np.pi * np.arange(1, 8).reshape(1, 1, 7, 1) * phi2 / 8.0).reshape(16, 14, 8)
    w = np.concatenate([w2, w3], 1).reshape(16 * 29, 8)
    w = np.concatenate([w.real, w.imag], 1)
    return np.ascontiguousarray(np.broadcast_to(w[:, :, None], (16 * 29, 16, 128)), dtype=np.float32)


def _cmul(a, w):
    return (a[0] * w[0] - a[1] * w[1], a[0] * w[1] + a[1] * w[0])


def _cmul_conj(a, w):
    return (a[0] * w[0] + a[1] * w[1], a[1] * w[0] - a[0] * w[1])


def _crot(a, k, n):
    k %= n
    if k == 0:
        return a
    c, s = math.cos(2 * math.pi * k / n), math.sin(2 * math.pi * k / n)
    if (8 * k) % n == 0 and (4 * k) % n:
        if c * s > 0:
            return ((a[0] - a[1]) * c, (a[0] + a[1]) * c)
        return ((a[0] + a[1]) * c, (a[1] - a[0]) * c)
    return _cmul(a, (c, s))


def _dft(get, idx, sign, cin=0, put=None, cout=0):
    n = len(idx)
    if n == 1:
        a = get(idx[0])
        yield cin
        return [a]
    if n == 2:
        a, b = get(idx[0]), get(idx[1])
        if a[1] is None:
            y = [(a[0] + b[0], b[1]), (a[0] - b[0], -b[1])]
        else:
            y = [(a[0] + b[0], a[1] + b[1]), (a[0] - b[0], a[1] - b[1])]
        yield 2 * cin + 4
        return y
    e = yield from _dft(get, idx[0::2], sign, cin)
    o1 = yield from _dft(get, idx[1::4], sign, cin)
    o3 = yield from _dft(get, idx[3::4], sign, cin)
    y = [None] * n
    for k in range(n // 4):
        a, b = _crot(o1[k], sign * k, n), _crot(o3[k], 3 * sign * k, n)
        p = (a[0] + b[0], a[1] + b[1])
        m = (a[0] - b[0], a[1] - b[1])
        e0, e1 = e[k], e[k + n // 4]
        y[k] = (e0[0] + p[0], e0[1] + p[1])
        y[k + n // 2] = (e0[0] - p[0], e0[1] - p[1])
        up = (e1[0] - m[1], e1[1] + m[0])
        dn = (e1[0] + m[1], e1[1] - m[0])
        y[k + n // 4], y[k + 3 * n // 4] = (up, dn) if sign > 0 else (dn, up)
        if put is not None:
            for j in range(k, n, n // 4):
                put(j, y[j])
        yield 12 + (0 if k == 0 else 8 if 8 * k == n else 12) + 4 * cout
    return y


def _fft_first(src, dst, st, g, row):
    def get(n):
        a = src[g, pl.ds(FB * n + row, 8), :]
        return (a * math.cos(math.pi * n / 32), a * math.sin(math.pi * n / 32)) if n else (a, None)

    def put(j, y):
        for z in range(2):
            st.add(dst, (z, g, pl.ds(FB * j + row, 8)), y[z])
    return 200, (src, dst), _dft(get, list(range(16)), 1, 2, put)


def _fft_middle(fu, fh, work, st, tw, g, b):
    twiddle = lambda i: (tw[b * 29 + i, 0:8], tw[b * 29 + i, 8:16])
    w2 = lambda n: twiddle(n - 1)
    w3 = lambda half, n: twiddle(14 + 7 * half + n)

    def save(area, exchange):
        def put(i, y):
            for z in range(2):
                row = EX0 + ((2 * area + z) * 16 + i) * ST if exchange else HO0 + _low(32 * area + 2 * i + z)
                st.add(work, (pl.ds(row, 8),), y[z], tag=(area, exchange))
        return put

    def saved(area, i):
        return tuple(work[pl.ds(HO0 + _low(32 * area + 2 * i + z), 8), :] for z in range(2))

    def exchanged(area, i):
        return tuple(work[pl.ds(EX0 + ((2 * area + z) * 16 + i // 8 * 8) * ST + i % 8, 8, stride=ST), :]
                     for z in range(2))

    def pass1(s, src):
        def get(n):
            a = tuple(src[z, g, pl.ds(b * FB + 8 * n, 8), :] for z in range(2))
            return _cmul(a, w2(n)) if n else a
        for m in range(4):
            put = lambda k, y: save(s, False)(4 * m + k, y if (m * k) % 4 == 0 else _crot(y, m * k, 16))
            yield from _dft(get, list(range(m, 16, 4)), 1, 6, put, (0, 4, 2, 4)[m])

    def pass2(s):
        st.flush((s, False))
        put = save(s, True)
        for k in range(4):
            x = [saved(s, 4 * m + k) for m in range(4)]
            if k == 2:
                e = [(x[0][0] - x[2][1], x[0][1] + x[2][0]), (x[0][0] + x[2][1], x[0][1] - x[2][0])]
            else:
                e = [(x[0][0] + x[2][0], x[0][1] + x[2][1]), (x[0][0] - x[2][0], x[0][1] - x[2][1])]
            p = (x[1][0] + x[3][0], x[1][1] + x[3][1])
            q = (x[1][0] - x[3][0], x[1][1] - x[3][1])
            put(k, (e[0][0] + p[0], e[0][1] + p[1]))
            put(k + 8, (e[0][0] - p[0], e[0][1] - p[1]))
            yield 16
            put(k + 4, (e[1][0] - q[1], e[1][1] + q[0]))
            put(k + 12, (e[1][0] + q[1], e[1][1] - q[0]))
            yield 12

    def spectrum(s, half, put, cout):
        st.flush((s, True))
        get = lambda n: _cmul(exchanged(s, 8 * half + n), w3(half, n)) if n else exchanged(s, 8 * half)
        yield from _dft(get, list(range(8)), 1, 6, put, cout)

    def product(half):
        st.flush((2 + half, False))
        prod = {}
        yield from spectrum(1, half, lambda j, y: prod.update({j: _cmul(saved(2 + half, j), y)}), 6)
        put = lambda n, y: save(2, True)(8 * half + n, _cmul_conj(y, w3(half, n)) if n else y)
        yield from _dft(prod.get, list(range(8)), -1, 0, put, 6)

    def inverse():
        def put(n, y):
            a = _cmul_conj(y, w2(n)) if n else y
            for z in range(2):
                st.add(fu, (z, g, pl.ds(b * FB + 8 * n, 8)), a[z])
        st.flush((2, True))
        yield from _dft(lambda j: exchanged(2, j), list(range(16)), -1, 0, put, 6)

    forward = [(200, (src,), pass1(s, src)) for s, src in enumerate((fu, fh))]
    forward += [(112, (), pass2(s)) for s in range(2)]
    forward += [(104, (), spectrum(0, half, save(2 + half, False), 0)) for half in range(2)]
    forward += [(256, (), product(half)) for half in range(2)]
    return forward, (264, (fu,), inverse())


def _fft_last(src, dst, st, g, row):
    def put(n, y):
        a = y[0] * (math.cos(math.pi * n / 32) / S)
        st.add(dst, (g, pl.ds(FB * n + row, 8)), a + y[1] * (math.sin(math.pi * n / 32) / S) if n else a)
    get = lambda j: tuple(src[z, g, pl.ds(FB * j + row, 8), :] for z in range(2))
    return 216, (src, dst), _dft(get, list(range(16)), -1, 0, put, 3)


def _kernel(x_hbm, wqkv_hbm, wo_hbm, k_hbm, v_hbm, ssm_hbm, tw_hbm, shift_hbm, dvec_hbm, gate_hbm, out_hbm,
            x_v, w_v, wo_v, k_v, v_v, ssm_v, tw_v, out_v, kg, qh, vt, ot, u_s, h_s, fu, fh, k32, q32,
            work, pb0, pb1, qw, kf, o_first, wt, gate_s, shift_v, dvec_v, gate_v, zero_s, sems, osems):
    st = _Stores()
    slow = 7
    lead = 200
    runtime_zero = lambda i: pl.multiple_of(16 * (i >> 6), 16)

    copies = []

    def copy(src, dst):
        copies.append(pltpu.make_async_copy(src, dst, sems.at[len(copies)]))
        return copies[-1]

    rows_copy = lambda src, dst, start, size: copy(src.at[pl.ds(start, size)], dst.at[pl.ds(start, size)])
    cp_x = [rows_copy(x_hbm, x_v, sum(KROWS[:i]), n) for i, n in enumerate(KROWS)]
    cp_w = [copy(wqkv_hbm.at[:, pl.ds(i * D, D)], w_v.at[i]) for i in range(3)]
    cp_k = [rows_copy(k_hbm, k_v, r, S // 2) for r in (0, S // 2)]
    cp_v = [rows_copy(v_hbm, v_v, r, S // 2) for r in (0, S // 2)]
    cp_ssm = [rows_copy(ssm_hbm, ssm_v, 0, D - 128), rows_copy(ssm_hbm, ssm_v, D - 128, 128)]
    cp_tw = copy(tw_hbm, tw_v.at[:, pl.ds(0, 16)])
    cp_wo = copy(wo_hbm, wo_v)
    cp_small = [copy(shift_hbm, shift_v.at[:, pl.ds(0, D)]), copy(dvec_hbm, dvec_v), copy(gate_hbm, gate_v)]

    def wait(*cps):
        for cp in cps:
            cp.wait()

    for cp in (*cp_small, cp_w[1], *cp_x, cp_w[0], cp_ssm[0], cp_k[0], cp_v[0], cp_w[2], cp_ssm[1],
               cp_k[1], cp_v[1], cp_tw, cp_wo):
        cp.start()

    def clear(i, _):
        row = pl.multiple_of(_top(i, 0), 16)
        pb1.bitcast(U32)[pl.ds(row, 16), :] = jnp.zeros((16, 128), U32)
        for half in range(2):
            qw[pl.ds(row + 32 * 64 * half, 16), :] = jnp.zeros((16, 128), U32)
        zero_s[0] = i >> 6
    lax.fori_loop(0, 64, clear, None)
    ot[0, :, pl.ds(S - BQ, BQ)] = jnp.zeros((DV, BQ), F32)

    def weight_block(n, i, j):
        st.add(wt, (n, j, pl.ds(128 * i, 128)), w_v[2 * n, pl.ds(128 * j, 128), pl.ds(128 * i, 128)].T, slow)
        yield 40

    def gate_block(r):
        xf = x_v[pl.ds(r, 64), :].astype(F32)
        logit = jnp.sum(xf * gate_v[...].astype(F32).reshape(1, D), axis=-1, keepdims=True)
        st.add(gate_s, (pl.ds(r, 64),), jnp.broadcast_to(jax.nn.sigmoid(logit), (64, 128)), slow)
        yield 200

    weights = lambda n: [(40, (wt,)[n:], weight_block(n, i, j)) for i in range(G) for j in range(G)]
    gates = lambda i: [(200, (gate_s,), gate_block(r)) for r in range(sum(KROWS[:i]), sum(KROWS[:i + 1]), 64)]
    last_group = lambda h: (DH * h + DH - 1) >> 7

    def key_group(h):
        first = (DH * h) >> 7
        return first + G * (last_group(h) - first)

    def project_k(block, items):
        r0, n = sum(KROWS[:block]), KROWS[block]
        rest = [_dot(x_v[pl.ds(r0 + i * n // 4, n // 4), 512:], w_v[1, 512:, 512:]) for i in range(4)]
        rest = jnp.concatenate([_dot(x_v[pl.ds(r0, n), 512:], w_v[1, 512:, :512]), jnp.concatenate(rest, 0)], 1)
        groups = [_dot(x_v[pl.ds(r0, n), :512], w_v[1, :512, 128 * g:128 * g + 128]) + rest[:, 128 * g:128 * g + 128]
                  for g in range(G)]
        groups = [val * (DH ** -0.5 * math.log2(math.e)) for val in groups]
        left = lax.broadcasted_iota(jnp.int32, (n, 128), 1) < 64
        groups += [jnp.where(left, groups[g + 1], groups[g]) for g in range(G - 1)]
        for g in (0, 1, 5, 2, 6, 3, 7, 4, 8):
            for r in range(n // 16):
                kg[g, pl.ds(2 * _low(r0 // 16 + r), 16), :] = groups[g][16 * r:16 * r + 16].astype(BF16)
        side = _SideWork(items, st, runtime_zero(zero_s[0]))
        for g in range(G + 1):
            ready = [(h, j) for j in range(n // BK) for h in range(NA) if last_group(h) == g - 1]
            for i in range(8):
                for h, j in ready[i * len(ready) // 8:(i + 1) * len(ready) // 8]:
                    val = groups[key_group(h)][BK * (j + 1) - NV:BK * (j + 1)]
                    k32[h, r0 // BK + j, :NV] = pltpu.roll(val, -DH * h % 128, 1) if h and g < G else val
                if g < G:
                    tick = groups[g][i * n // 8:i * n // 8 + 16]
                    side.pin(k32, tick)
                    side.run_to(side.total * (8 * g + i + 1) / 30, tick)
        side.finish()

    wait(*cp_small, cp_w[1], cp_x[0])
    project_k(0, gates(0))
    wait(cp_x[1])
    project_k(1, gates(1))
    wait(cp_x[2])
    project_k(2, gates(2))
    wait(cp_x[3], cp_w[0])
    project_k(3, weights(0))

    def project_t(n, chunks, emit, items):
        side = _SideWork(items, st, runtime_zero(zero_s[0]))
        side.run_to(lead)
        weight = lambda j: pltpu.bitcast(wt.bitcast(U32)[n, j, :D // 2], BF16)
        ticks, count = len(chunks) * (XC // 128 + 1) * (D // 32), 0

        def pace(val):
            nonlocal count
            for r in range(0, D, 32):
                count += 1
                side.run_to(lead + (side.total - lead) * 1.02 * count / ticks, val[r:r + 16, 0:128])

        for c in chunks:
            rest = _dot_nt(weight(G - 1), x_v[pl.ds(c * XC, XC), 512:])
            pace(rest)
            for z in range(XC // 128):
                val = _dot_nt(jnp.concatenate([weight(j) for j in range(G - 1)], 1),
                              x_v[pl.ds(c * XC + 128 * z, 128), :512]) + rest[:, 128 * z:128 * z + 128]
                emit(c * XC // 128 + z, val)
                pace(val)
        side.finish()

    sub = lax.broadcasted_iota(jnp.int32, (8, 128), 0)

    def emit_q(z, val):
        q32[pl.ds(z * D, NA * DH), :] = val[:NA * DH]
        for h in range(H):
            lo, hi = DH * h, DH * (h + 1)
            parts = []
            for r in range(lo // 16 * 16, lo // 16 * 16 + 32, 8):
                part = val[r:r + 8]
                parts.append(jnp.zeros((8, 128), F32) if r + 8 <= lo or r >= hi else
                             jnp.where(sub >= lo - r, part, 0.0) if r < lo else
                             jnp.where(sub < hi - r, part, 0.0) if r + 8 > hi else part)
            qh[h, pl.ds(32 * z, 32), :] = jnp.concatenate(parts, 0).astype(BF16)

    def emit_v(z, val):
        for h in range(0, H, 2):
            r = DH * h
            mid = val[r + 16:r + 24]
            vt[h, pl.ds(32 * z, DV), :] = jnp.concatenate([val[r:r + 16], jnp.where(sub < 4, mid, 1.0)], 0)
            vt[h + 1, pl.ds(32 * z, DV), :] = jnp.concatenate([jnp.where(sub < 4, 1.0, mid), val[r + 24:r + 40]], 0)

    def filter_block(g, z):
        st.add(h_s, (g, pl.ds(z * FB, 128)), ssm_v[pl.ds(128 * g, 128), pl.ds(128 * z, 128)].astype(F32).T, slow)
        yield 40

    def signal_block(g, z):
        cols = pl.ds(128 * g, 128)
        w = shift_v[:, cols].astype(F32)
        base = z % 2 * FB
        stage = kf.at[pl.ds(runtime_zero(zero_s[0]), 2 * FB)]
        stage[pl.ds(base, 8), :] = k_v[pl.ds(128 * z - 16, 16), cols].astype(F32)[8:] if z else jnp.zeros((8, 128), F32)
        stage[pl.ds(base + 8, 128), :] = k_v[pl.ds(128 * z, 128), cols].astype(F32)
        yield 40
        for r in range(0, 128, 32):
            acc = kf[pl.ds(base + 8 + r, 32), :] * w[0:1]
            for t in range(1, KS):
                acc = acc + kf[pl.ds(base + 8 + r - t, 32), :] * w[t:t + 1]
            st.add(u_s, (g, pl.ds(z * FB + r, 32)), acc * v_v[pl.ds(128 * z + r, 32), cols].astype(F32))
            yield 44

    def stores_done():
        st.flush()
        yield 0

    filters = lambda g: [(40, (h_s,), filter_block(g, z)) for z in range(16)]
    signals = lambda i: [(216, (kf, u_s), signal_block(g, z)) for g in range(G) for z in range(8 * i, 8 * i + 8)]
    first = lambda src, dst, g: [(0, (), stores_done())] + [_fft_first(src, dst, st, g, r) for r in range(0, 128, 8)]

    wait(cp_ssm[0])
    items = filters(0)
    for i, item in enumerate(gates(3)):
        items.insert(3 * i, item)
    for g in range(3):
        passes = first(h_s, fh, g)
        for i, item in enumerate(filters(g + 1)):
            passes.insert(1 + i + i * 3 // 4, item)
        items += passes
    project_t(0, (0, 1), emit_q, items)
    wait(cp_k[0], cp_v[0], cp_w[2], cp_ssm[1])
    items = filters(4)
    project_t(0, (2, 3), emit_q, first(h_s, fh, 3) + items[:1]
              + [item for pair in zip(signals(0), weights(1) + items[1:], strict=True) for item in pair])

    kg32, qh32 = kg.bitcast(U32), qh.bitcast(U32)
    kb_row = lambda j, i, d: _low(((j * (NV // 16) + i // 2) * DH + d) * 2 + i % 2)
    qb_row = lambda z, d: _top(z // 2 * DH + d, z)
    p_row = lambda r, z: 2 * _top(r * NZ + z, z + min(r // 8, 1))

    def spread_keys(h, j, d, nv):
        col = jnp.broadcast_to(k32[h, j, NV - nv:NV, d:d + 1], (nv, 128))
        for i in range(nv // 8):
            work[pl.ds(kb_row(j, (NV - nv) // 8 + i, d), 8), :] = col[8 * i:8 * i + 8]

    def spread_query(h, z, d):
        work[pl.ds(qb_row(z, d), 8), :] = jnp.broadcast_to(q32[pl.ds(z * D + DH * h + d, 1), :], (8, 128))

    def stage_queries(h, z):
        slot = lambda r: pl.ds(pl.multiple_of(_top(8 * z + (r & 7), z), 8), 8)
        for i in range(2):
            qw[slot(((DH * jnp.maximum(h - 1, 0)) >> 4) + i), :] = jnp.zeros((8, 128), U32)
        for i in range(2):
            qw[slot(((DH * h) >> 4) + i), :] = qh32[h, pl.ds(16 * z + 8 * i, 8), :]

    def query_tiles(z0, n):
        tiles = [jnp.concatenate([qw[pl.ds(_top(8 * z + r, z), 8), :] for r in range(8)], 0) for z in range(z0, z0 + n)]
        return pltpu.bitcast(jnp.concatenate(tiles, 1), BF16)

    def key_rows(grp, r0, n):
        return pltpu.bitcast(jnp.concatenate([kg32[grp, pl.ds(_low(r), 8), :] for r in range(r0, r0 + n)], 0), BF16)

    def value_tiles(h, k0, n):
        return jnp.concatenate([vt[h, pl.ds(32 * k, DV), :] for k in range(k0, k0 + n)], 1)

    def late_keys():
        for h in range(NA):
            if last_group(h) == G - 1:
                for j in range(NK):
                    k32[h, j, :NV] = pltpu.roll(k32[h, j, :NV], -DH * h % 128, 1)
                    yield 10

    def first_operands():
        for d in range(DH):
            spread_keys(0, 0, d, NV)
            yield 20
        for z in range((NQ - 1) * NZ):
            stage_queries(0, z)
        for z in range(2 * NZ):
            for d in range(DH):
                spread_query(0, z, d)
            yield 40

    wait(cp_k[1], cp_v[1])
    project_t(1, (0, 1, 2, 3), emit_v,
              [(80, (), late_keys())] + first(h_s, fh, 4) + [(720, (work,), first_operands())] + signals(1)
              + [item for g in range(G) for item in first(u_s, fu, g)])
    wait(cp_tw)

    def vpu_scores(a, j, pair, z0, slot, p_out):
        acc = [None, None]
        for d in range(DH):
            keys = jnp.concatenate([work[pl.ds(kb_row(j, 2 * pair + i, d), 8), :] for i in range(2)], 0)
            for i in range(2):
                qrow = work[pl.ds(qb_row(a * NZ + z0 + i, d), 8), :]
                term = keys * jnp.concatenate([qrow, qrow], 0)
                acc[i] = acc[i] + term if d else term
            if d == DH - 1:
                for i in range(2):
                    p_out[pl.ds(p_row(slot, z0 + i), 16), :] = jnp.exp2(acc[i]).astype(BF16)
            yield

    def weighted_values(h, t, nv):
        src = (pb0, pb1)[t % 2].bitcast(U32)
        slots = [BK // 16 if nv == NV and r == (BK - NV) // 16 else r for r in range(BK // 16)]
        p = [jnp.concatenate([src[pl.ds(p_row(r, z) // 2, 8), :] for r in slots], 0) for z in range(NZ)]
        return _dot(value_tiles(h, STEPS[t][1] * BK // 128, BK // 128), pltpu.bitcast(jnp.concatenate(p, 1), BF16))

    def head(h, items):
        is_last, shared = isinstance(h, int), not items
        side = _SideWork(items, st, runtime_zero(zero_s[0] if is_last else h))
        grp, nxt = key_group(h), jnp.minimum(h + 1, NA - 1)
        nvs = VPU_KEYS if shared else [0] * len(STEPS)
        pv_span = 52 if shared else 36
        p_outs = [pb.at[pl.ds(side.zero, pb.shape[0] - 64)] for pb in (pb0, pb1)]
        blocks, due = [], []
        for t, (a, j) in enumerate(STEPS):
            if shared:
                blocks += [(a, j, pair, z0, (BK - NV) // 16 + pair, p_outs[t % 2]) for pair in (1, 2) for z0 in (0, 2)]
            due.append(DH * len(blocks))
            if a % 2 == 0 and nvs[NQ * j + NQ - 1] == NV:
                blocks.append((NQ - 1, j, 0, a, BK // 16, p_outs[1]))
                due[-1] += DH // 2
        scores, scored = (None for block in blocks for _ in vpu_scores(*block)), 0
        side.run_to(lead)
        if shared:
            for z in range(2 * NZ, NQ * NZ):
                for d in range(DH):
                    spread_query(h, z, d)
        acc, res = {}, None
        for t, (a, j) in enumerate(STEPS):
            rows = BK - nvs[t]
            s = _dot(key_rows(grp, j * BK // 16, rows // 16), query_tiles(a * NZ, NZ))
            if t:
                side.pin(qw, res[0:8, 0:128])
            if t == 0 or (t > len(STEPS) - NQ and not is_last):
                for z in range(NZ):
                    stage_queries(h + 1 if t else h, (a - 1) % NQ * NZ + z)

            def advance(tick, clock, begin=scored):
                nonlocal scored
                frac = clock / (rows + pv_span)
                while scored < begin + (due[t] - begin) * frac - 0.500001:
                    next(scores)
                    scored += 1
                side.run_to(lead + (side.total - lead) * (t + frac) / len(STEPS), tick)

            for r in range(rows // 16):
                for z in range(NZ):
                    p_outs[t % 2][pl.ds(p_row(r, z), 16), :] = jnp.exp2(
                        s[16 * r:16 * r + 16, 128 * z:128 * z + 128]).astype(BF16)
                tick = s[16 * r:16 * r + 8, 0:128]
                side.pin(work, tick)
                if shared and r % 3 == 0:
                    jn = (j + 1) % NK
                    spread_keys(h if jn else nxt, jn, a * DH // NQ + r // 3, max(nvs[NQ * jn:NQ * jn + NQ]))
                if shared and t >= len(STEPS) - 2 and r < 14:
                    for i in range(r * NZ * DH // 14, (r + 1) * NZ * DH // 14):
                        spread_query(nxt, (t - len(STEPS) + 2) * NZ + i // DH, i % DH)
                advance(tick, 16 * (r + 1))
            if t == 0:
                res = weighted_values(jnp.maximum(h - 1, 0), len(STEPS) - 1, 0)
                ot[h, :, pl.ds(S - BQ, BQ)] += res
            else:
                a, j = STEPS[t - 1]
                res = weighted_values(h, t - 1, nvs[t - 1])
                acc[a] = acc[a] + res if j else res
                if t + NQ >= len(STEPS):
                    ot[h + 1, :, pl.ds(a * BQ, BQ)] = acc[a]
            for i, tick in enumerate((res[0:8, 0:128], res[16:24, 0:128], res[8:16, 256:384])):
                side.pin(work, tick)
                advance(tick, rows + pv_span * (i + 1) / 3)
            assert scored == due[t]
        side.finish()

    def middle(g):
        items, back = [], []
        for b in range(16):
            forward, inverse = _fft_middle(fu, fh, work, st, tw_v, g, b)
            items += forward[:1] + back + forward[1:]
            back = [inverse]
        return items + back

    lax.fori_loop(0, NA, lambda h, _: head(h, []), None)
    lax.fori_loop(0, NM, lambda g, _: head(NA + g, middle(g)), None)
    head(H - 1, [_fft_last(fu, h_s, st, g, r) for g in range(G) for r in range(0, 128, 8)])

    def normalize(z):
        cols = pl.ds(_aligned(z * 128, 128), 128)
        parts, lo, hi = [], None, None
        for h in range(0, H, 2):
            even, odd = ot[h + 1, :, cols], ot[h + 2, :, cols]
            denom = jnp.where(sub < 4, odd[0:8], even[16:24])
            lo, hi = (jnp.minimum(lo, denom), jnp.maximum(hi, denom)) if h else (denom, denom)
            inv = 1.0 / denom
            ie, io = inv[4:5], inv[0:1]
            parts += [even[0:16] * ie, jnp.where(sub < 4, even[16:24] * ie, odd[0:8] * io), odd[8:24] * io]
        return jnp.concatenate(parts, 0).T.astype(BF16), jnp.where((lo >= L_LO) & (hi <= L_HI), 0.0, 1.0)

    def mix(z0, o):
        n = o.shape[0]
        rows = pl.ds(_aligned(z0 * 128, 128), n)
        a = _dot(o, wo_v[...])
        gate = jnp.concatenate([gate_s[rows, :]] * G, 1)
        plane = lambda ref: jnp.concatenate([jnp.concatenate(
            [ref[g, pl.ds(_aligned((z0 + z) * FB, 8), 128), :] for z in range(n // 128)], 0) for g in range(G)], 1)
        b = x_v[rows, :].astype(F32) * (plane(h_s) + plane(u_s) * dvec_v[...].astype(F32).reshape(1, D))
        out_v[rows, :] = (gate * a + (1.0 - gate) * b).astype(BF16)

    def out_copy(r0, n, sem):
        return pltpu.make_async_copy(out_v.at[pl.ds(r0, n)], out_hbm.at[pl.ds(r0, n)], osems.at[sem])

    ot[H, :, pl.ds(S - BQ, BQ)] += weighted_values(H - 1, len(STEPS) - 1, 0)
    o_first[...], unsafe = normalize(0)
    wait(cp_wo)
    cp_out = [out_copy(sum(OUT[:i]), n, i) for i, n in enumerate(OUT)]
    for i, n in enumerate(OUT):
        z = sum(OUT[:i]) // 128
        if i:
            o, flags = zip(*[normalize(z + e) for e in range(n // 128)])
            unsafe = unsafe + sum(flags)
        mix(z, jnp.concatenate(o, 0) if i else o_first[...])
        cp_out[i].start()
    unsafe = jnp.max(unsafe)
    wait(*cp_out)

    @pl.when(unsafe > 0.0)
    def _():
        def attend(i, _):
            h, z = i // (S // 128), i % (S // 128)
            for r in range(8):
                qw[pl.ds(_top(r, 0), 8), :] = jnp.zeros((8, 128), U32)
            for r in range(2):
                qw[pl.ds(pl.multiple_of(_top((((DH * h) >> 4) + r) & 7, 0), 8), 8), :] = (
                    qh32[h, pl.ds(pl.multiple_of(16 * z + 8 * r, 8), 8), :])
            s = _dot(key_rows(key_group(h), 0, S // 16), query_tiles(0, 1))
            p = jnp.exp2(s - jnp.max(s, axis=0, keepdims=True)).astype(BF16)
            ot[h + 1, :, pl.ds(pl.multiple_of(z * 128, 128), 128)] = _dot(value_tiles(h, 0, S // 128), p)
        lax.fori_loop(0, H * (S // 128), attend, None)
        lax.fori_loop(0, S // 128, lambda z, _: mix(z, normalize(z)[0]), None)
        whole = out_copy(0, S, 0)
        whole.start()
        whole.wait()


@jax.jit
def pallas_gated_mix__mha_block__ssm_conv_h3__prompt_kernel(
    A_x: jax.Array,
    A_wqkv: jax.Array,
    A_wo: jax.Array,
    B_q: jax.Array,
    B_k: jax.Array,
    B_v: jax.Array,
    B_shift_k: jax.Array,
    B_ssm_k: jax.Array,
    B_ssm_D: jax.Array,
    gate_w: jax.Array,
):
    del B_q
    tw = _twiddle_table()
    hbm = pl.BlockSpec(memory_space=pl.ANY)
    vmem = pltpu.VMEM
    out = pl.pallas_call(
        _kernel,
        in_specs=[hbm] * 10,
        out_specs=hbm,
        out_shape=jax.ShapeDtypeStruct((S, D), BF16),
        scratch_shapes=[
            vmem((S, D), BF16), vmem((3, D, D), BF16), vmem((D, D), BF16),
            vmem((S, D), BF16), vmem((S, D), BF16), vmem((D, S), BF16),
            vmem((tw.shape[0], 32, 128), F32), vmem((S, D), BF16),
            vmem((2 * G - 1, 2 * _low(S // 16), 128), BF16),
            vmem((H, S // 4, 128), BF16), vmem((H, S // 4, 128), F32),
            vmem((H + 1, DV, S), F32),
            vmem((G, 16 * FB, 128), F32), vmem((G, 16 * FB, 128), F32),
            vmem((2, G, 16 * FB, 128), F32), vmem((2, G, 16 * FB, 128), F32),
            vmem((NA, NK, NV + 16, 128), F32), vmem((S // 128 * D, 128), F32),
            vmem((WORK_ROWS, 128), F32),
            vmem((4 * NZ * (BK + 16) + 64, 128), BF16),
            vmem((4 * NZ * (BK + 16) + 64, 128), BF16),
            vmem((2 * S + 32, 128), U32), vmem((2 * FB + 16, 128), F32),
            vmem((128, D), BF16), vmem((2, G, D + 64, 128), BF16),
            vmem((S + 32, 128), F32),
            vmem((KS, 1536), BF16), vmem((D,), BF16), vmem((D,), BF16),
            pltpu.SMEM((1,), jnp.int32),
            pltpu.SemaphoreType.DMA((18,)), pltpu.SemaphoreType.DMA((len(OUT),)),
        ],
        compiler_params=pltpu.CompilerParams(vmem_limit_bytes=124 * 2 ** 20),
    )(A_x.reshape(S, D), A_wqkv, A_wo, B_k.reshape(S, D), B_v.reshape(S, D), B_ssm_k, tw,
      B_shift_k.T, B_ssm_D, gate_w)
    return out.reshape(1, S, D)
```

```python
import math

import jax
import jax.numpy as jnp
import numpy as np
from jax import lax
import jax.experimental.pallas as pl
import jax.experimental.pallas.tpu as pltpu

S, D, H, KS = 2048, 640, 32, 4
DH = D // H
G = D // 128
F32, BF16, U32 = jnp.float32, jnp.bfloat16, jnp.uint32

XC = 512
BQ, BK = 512, 256
NZ, NQ, NK = BQ // 128, S // BQ, S // BK
STEPS = [(a, j) for j in range(NK) for a in range(NQ)]
DV = 24
NM, NL = G, 1
NA = H - NM - NL
NV = 48
VPU_KEYS = [[NV if a == NQ - 1 and j < NK - e else 32 for a, j in STEPS] for e in range(2)]
QUERY_TICKS = (1, 4, 7, 10, 11)
OUT = [128, 256, 256, 256, 256, 256, 256, 256, 128]
KROWS = [256, 512, 768, 512]
L_LO, L_HI = 2.0 ** -30, 2.0 ** 30

ST = 9
FB = 136


def _low(i):
    return 8 * (i + i // 2 * 2)


def _top(i, bank):
    return 32 * i + 16 + 8 * (bank % 2)


EX0 = _low(NK * DH * NV // 8)
HO0 = EX0 + 6 * 16 * ST
WORK_ROWS = HO0 + _low(128) + 32


def _dot(a, b):
    return lax.dot_general(a, b, (((1,), (0,)), ((), ())), preferred_element_type=F32)


def _dot_nt(a, b):
    return lax.dot_general(a, b, (((1,), (1,)), ((), ())), preferred_element_type=F32)


def _aligned(start, align):
    return start if isinstance(start, int) else pl.multiple_of(start, align)


class _Stores:
    def __init__(self):
        self.pending = []

    def add(self, ref, idx, val, delay=3, tag=None):
        self.pending.append([delay, tag, ref, idx, val])

    def _emit(self, ready):
        for item in self.pending:
            if ready(item):
                item[2][item[3] + (slice(None),)] = item[4]
        self.pending = [item for item in self.pending if not ready(item)]

    def tick(self):
        for item in self.pending:
            item[0] -= 1
        self._emit(lambda item: item[0] <= 0)

    def flush(self, tag=None):
        self._emit(lambda item: tag is None or item[1] == tag)


class _SideWork:
    def __init__(self, items, stores, zero):
        self.items, self.stores, self.zero = list(items), stores, zero
        self.total, self.done = sum(item[0] for item in items), 0

    def pin(self, ref, val):
        val = val.astype(BF16) if ref.dtype == BF16 else pltpu.bitcast(val[:8], ref.dtype)
        rows = pl.ds(self.zero + ref.shape[-2] - val.shape[0], val.shape[0])
        ref[(0,) * (len(ref.shape) - 2) + (rows, slice(None))] = val

    def run_to(self, goal, tick=None):
        pinned = []
        while self.items and self.done < goal:
            for ref in self.items[0][1]:
                if tick is not None and not any(ref is other for other in pinned):
                    self.pin(ref, tick)
                    pinned.append(ref)
            cost = next(self.items[0][2], None)
            if cost is None:
                self.items.pop(0)
            else:
                self.done += cost
        self.stores.tick()

    def finish(self):
        self.run_to(math.inf)
        self.stores.flush()


def _twiddle_table():
    phi1 = (0.25 + np.arange(16)[:, None]) / 16.0
    w2 = np.exp(2j * np.pi * np.arange(1, 16)[None, :] * phi1 / 16.0)
    w2 = np.broadcast_to(w2[:, :, None], (16, 15, 8))
    phi2 = ((phi1 + np.arange(16)[None, :]) / 16.0).reshape(16, 2, 1, 8)
    w3 = np.exp(2j * np.pi * np.arange(1, 8).reshape(1, 1, 7, 1) * phi2 / 8.0).reshape(16, 14, 8)
    w = np.concatenate([w2, w3], 1).reshape(16 * 29, 8)
    w = np.concatenate([w.real, w.imag], 1)
    return np.ascontiguousarray(np.broadcast_to(w[:, :, None], (16 * 29, 16, 128)), dtype=np.float32)


def _cmul(a, w):
    return (a[0] * w[0] - a[1] * w[1], a[0] * w[1] + a[1] * w[0])


def _cmul_conj(a, w):
    return (a[0] * w[0] + a[1] * w[1], a[1] * w[0] - a[0] * w[1])


def _crot(a, k, n):
    k %= n
    if k == 0:
        return a
    c, s = math.cos(2 * math.pi * k / n), math.sin(2 * math.pi * k / n)
    if (8 * k) % n == 0 and (4 * k) % n:
        if c * s > 0:
            return ((a[0] - a[1]) * c, (a[0] + a[1]) * c)
        return ((a[0] + a[1]) * c, (a[1] - a[0]) * c)
    return _cmul(a, (c, s))


def _dft(get, idx, sign, cin=0, put=None, cout=0):
    n = len(idx)
    if n == 1:
        a = get(idx[0])
        yield cin
        return [a]
    if n == 2:
        a, b = get(idx[0]), get(idx[1])
        if a[1] is None:
            y = [(a[0] + b[0], b[1]), (a[0] - b[0], -b[1])]
        else:
            y = [(a[0] + b[0], a[1] + b[1]), (a[0] - b[0], a[1] - b[1])]
        yield 2 * cin + 4
        return y
    e = yield from _dft(get, idx[0::2], sign, cin)
    o1 = yield from _dft(get, idx[1::4], sign, cin)
    o3 = yield from _dft(get, idx[3::4], sign, cin)
    y = [None] * n
    for k in range(n // 4):
        a, b = _crot(o1[k], sign * k, n), _crot(o3[k], 3 * sign * k, n)
        p = (a[0] + b[0], a[1] + b[1])
        m = (a[0] - b[0], a[1] - b[1])
        e0, e1 = e[k], e[k + n // 4]
        y[k] = (e0[0] + p[0], e0[1] + p[1])
        y[k + n // 2] = (e0[0] - p[0], e0[1] - p[1])
        up = (e1[0] - m[1], e1[1] + m[0])
        dn = (e1[0] + m[1], e1[1] - m[0])
        y[k + n // 4], y[k + 3 * n // 4] = (up, dn) if sign > 0 else (dn, up)
        if put is not None:
            for j in range(k, n, n // 4):
                put(j, y[j])
        yield 12 + (0 if k == 0 else 8 if 8 * k == n else 12) + 4 * cout
    return y


def _fft_first(src, dst, st, g, row):
    def get(n):
        a = src[g, pl.ds(FB * n + row, 8), :]
        return (a * math.cos(math.pi * n / 32), a * math.sin(math.pi * n / 32)) if n else (a, None)

    def put(j, y):
        for z in range(2):
            st.add(dst, (z, g, pl.ds(FB * j + row, 8)), y[z])
    return 200, (src, dst), _dft(get, list(range(16)), 1, 2, put)


def _fft_middle(fu, fh, work, st, tw, g, b):
    twiddle = lambda i: (tw[b * 29 + i, 0:8], tw[b * 29 + i, 8:16])
    w2 = lambda n: twiddle(n - 1)
    w3 = lambda half, n: twiddle(14 + 7 * half + n)

    def save(area, exchange):
        def put(i, y):
            for z in range(2):
                row = EX0 + ((2 * area + z) * 16 + i) * ST if exchange else HO0 + _low(32 * area + 2 * i + z)
                st.add(work, (pl.ds(row, 8),), y[z], tag=(area, exchange))
        return put

    def saved(area, i):
        return tuple(work[pl.ds(HO0 + _low(32 * area + 2 * i + z), 8), :] for z in range(2))

    def exchanged(area, i):
        return tuple(work[pl.ds(EX0 + ((2 * area + z) * 16 + i // 8 * 8) * ST + i % 8, 8, stride=ST), :]
                     for z in range(2))

    def pass1(s, src):
        def get(n):
            a = tuple(src[z, g, pl.ds(b * FB + 8 * n, 8), :] for z in range(2))
            return _cmul(a, w2(n)) if n else a
        for m in range(4):
            put = lambda k, y: save(s, False)(4 * m + k, y if (m * k) % 4 == 0 else _crot(y, m * k, 16))
            yield from _dft(get, list(range(m, 16, 4)), 1, 6, put, (0, 4, 2, 4)[m])

    def pass2(s):
        st.flush((s, False))
        put = save(s, True)
        for k in range(4):
            x = [saved(s, 4 * m + k) for m in range(4)]
            if k == 2:
                e = [(x[0][0] - x[2][1], x[0][1] + x[2][0]), (x[0][0] + x[2][1], x[0][1] - x[2][0])]
            else:
                e = [(x[0][0] + x[2][0], x[0][1] + x[2][1]), (x[0][0] - x[2][0], x[0][1] - x[2][1])]
            p = (x[1][0] + x[3][0], x[1][1] + x[3][1])
            q = (x[1][0] - x[3][0], x[1][1] - x[3][1])
            put(k, (e[0][0] + p[0], e[0][1] + p[1]))
            put(k + 8, (e[0][0] - p[0], e[0][1] - p[1]))
            yield 16
            put(k + 4, (e[1][0] - q[1], e[1][1] + q[0]))
            put(k + 12, (e[1][0] + q[1], e[1][1] - q[0]))
            yield 12

    def spectrum(s, half, put, cout):
        st.flush((s, True))
        get = lambda n: _cmul(exchanged(s, 8 * half + n), w3(half, n)) if n else exchanged(s, 8 * half)
        yield from _dft(get, list(range(8)), 1, 6, put, cout)

    def product(half):
        st.flush((2 + half, False))
        prod = {}
        yield from spectrum(1, half, lambda j, y: prod.update({j: _cmul(saved(2 + half, j), y)}), 6)
        put = lambda n, y: save(2, True)(8 * half + n, _cmul_conj(y, w3(half, n)) if n else y)
        yield from _dft(prod.get, list(range(8)), -1, 0, put, 6)

    def inverse():
        def put(n, y):
            a = _cmul_conj(y, w2(n)) if n else y
            for z in range(2):
                st.add(fu, (z, g, pl.ds(b * FB + 8 * n, 8)), a[z])
        st.flush((2, True))
        yield from _dft(lambda j: exchanged(2, j), list(range(16)), -1, 0, put, 6)

    forward = [(200, (src,), pass1(s, src)) for s, src in enumerate((fu, fh))]
    forward += [(112, (), pass2(s)) for s in range(2)]
    forward += [(104, (), spectrum(0, half, save(2 + half, False), 0)) for half in range(2)]
    forward += [(256, (), product(half)) for half in range(2)]
    return forward, (264, (fu,), inverse())


def _fft_last(src, dst, st, g, row):
    def put(n, y):
        a = y[0] * (math.cos(math.pi * n / 32) / S)
        st.add(dst, (g, pl.ds(FB * n + row, 8)), a + y[1] * (math.sin(math.pi * n / 32) / S) if n else a)
    get = lambda j: tuple(src[z, g, pl.ds(FB * j + row, 8), :] for z in range(2))
    return 216, (src, dst), _dft(get, list(range(16)), -1, 0, put, 3)


def _kernel(x_hbm, wqkv_hbm, wo_hbm, k_hbm, v_hbm, ssm_hbm, tw_hbm, shift_hbm, dvec_hbm, gate_hbm, out_hbm,
            x_v, w_v, wo_v, k_v, v_v, ssm_v, tw_v, out_v, kg, qh, vt, ot, u_s, h_s, fu, fh, k32, q32,
            work, pb0, pb1, qw, kf, o_first, wt, gate_s, shift_v, dvec_v, gate_v, zero_s, sems, osems):
    st = _Stores()
    slow = 7
    lead = 200
    runtime_zero = lambda i: pl.multiple_of(16 * (i >> 6), 16)

    copies = []

    def copy(src, dst):
        copies.append(pltpu.make_async_copy(src, dst, sems.at[len(copies)]))
        return copies[-1]

    rows_copy = lambda src, dst, start, size: copy(src.at[pl.ds(start, size)], dst.at[pl.ds(start, size)])
    cp_x = [rows_copy(x_hbm, x_v, sum(KROWS[:i]), n) for i, n in enumerate(KROWS)]
    cp_w = [copy(wqkv_hbm.at[:, pl.ds(i * D, D)], w_v.at[i]) for i in range(3)]
    cp_k = [rows_copy(k_hbm, k_v, r, S // 2) for r in (0, S // 2)]
    cp_v = [rows_copy(v_hbm, v_v, r, S // 2) for r in (0, S // 2)]
    cp_ssm = [rows_copy(ssm_hbm, ssm_v, 0, D - 128), rows_copy(ssm_hbm, ssm_v, D - 128, 128)]
    cp_tw = copy(tw_hbm, tw_v.at[:, pl.ds(0, 16)])
    cp_wo = copy(wo_hbm, wo_v)
    cp_small = [copy(shift_hbm, shift_v.at[:, pl.ds(0, D)]), copy(dvec_hbm, dvec_v), copy(gate_hbm, gate_v)]

    def wait(*cps):
        for cp in cps:
            cp.wait()

    for cp in (*cp_small, cp_w[1], *cp_x, cp_w[0], cp_ssm[0], cp_k[0], cp_v[0], cp_w[2], cp_ssm[1],
               cp_k[1], cp_v[1], cp_tw, cp_wo):
        cp.start()

    def clear(i, _):
        row = pl.multiple_of(_top(i, 0), 16)
        pb1.bitcast(U32)[pl.ds(row, 16), :] = jnp.zeros((16, 128), U32)
        for half in range(2):
            qw[pl.ds(row + 32 * 64 * half, 16), :] = jnp.zeros((16, 128), U32)
        zero_s[0] = i >> 6
    lax.fori_loop(0, 64, clear, None)
    ot[NA - 1, :, pl.ds(S - BQ, BQ)] = jnp.zeros((DV, BQ), F32)

    def weight_block(n, i, j):
        st.add(wt, (n, j, pl.ds(128 * i, 128)), w_v[2 * n, pl.ds(128 * j, 128), pl.ds(128 * i, 128)].T, slow)
        yield 40

    def gate_block(r):
        xf = x_v[pl.ds(r, 64), :].astype(F32)
        logit = jnp.sum(xf * gate_v[...].astype(F32).reshape(1, D), axis=-1, keepdims=True)
        st.add(gate_s, (pl.ds(r, 64),), jnp.broadcast_to(jax.nn.sigmoid(logit), (64, 128)), slow)
        yield 200

    weights = lambda n: [(40, (wt,)[n:], weight_block(n, i, j)) for i in range(G) for j in range(G)]
    gates = lambda i: [(200, (gate_s,), gate_block(r)) for r in range(sum(KROWS[:i]), sum(KROWS[:i + 1]), 64)]
    last_group = lambda h: (DH * h + DH - 1) >> 7

    def key_group(h):
        first = (DH * h) >> 7
        return first + G * (last_group(h) - first)

    def project_k(block, items):
        r0, n = sum(KROWS[:block]), KROWS[block]
        rest = [_dot(x_v[pl.ds(r0 + i * n // 4, n // 4), 512:], w_v[1, 512:, 512:]) for i in range(4)]
        rest = jnp.concatenate([_dot(x_v[pl.ds(r0, n), 512:], w_v[1, 512:, :512]), jnp.concatenate(rest, 0)], 1)
        groups = [_dot(x_v[pl.ds(r0, n), :512], w_v[1, :512, 128 * g:128 * g + 128]) + rest[:, 128 * g:128 * g + 128]
                  for g in range(G)]
        groups = [val * (DH ** -0.5 * math.log2(math.e)) for val in groups]
        left = lax.broadcasted_iota(jnp.int32, (n, 128), 1) < 64
        groups += [jnp.where(left, groups[g + 1], groups[g]) for g in range(G - 1)]
        for g in (0, 1, 5, 2, 6, 3, 7, 4, 8):
            for r in range(n // 16):
                kg[g, pl.ds(2 * _low(r0 // 16 + r), 16), :] = groups[g][16 * r:16 * r + 16].astype(BF16)
        side = _SideWork(items, st, runtime_zero(zero_s[0]))
        for g in range(G + 1):
            ready = [(h, j) for j in range(n // BK) for h in range(NA) if last_group(h) == g - 1]
            for i in range(8):
                for h, j in ready[i * len(ready) // 8:(i + 1) * len(ready) // 8]:
                    val = groups[key_group(h)][BK * (j + 1) - NV:BK * (j + 1)]
                    k32[h, r0 // BK + j, :NV] = pltpu.roll(val, -DH * h % 128, 1) if h and g < G else val
                if g < G:
                    tick = groups[g][i * n // 8:i * n // 8 + 16]
                    side.pin(k32, tick)
                    side.run_to(side.total * (8 * g + i + 1) / 30, tick)
        side.finish()

    wait(*cp_small, cp_w[1], cp_x[0])
    project_k(0, gates(0))
    wait(cp_x[1])
    project_k(1, gates(1))
    wait(cp_x[2])
    project_k(2, gates(2))
    wait(cp_x[3], cp_w[0])
    project_k(3, weights(0))

    def project_t(n, chunks, emit, items):
        side = _SideWork(items, st, runtime_zero(zero_s[0]))
        side.run_to(lead)
        weight = lambda j: pltpu.bitcast(wt.bitcast(U32)[n, j, :D // 2], BF16)
        ticks, count = len(chunks) * (XC // 128 + 1) * (D // 32), 0

        def pace(val):
            nonlocal count
            for r in range(0, D, 32):
                count += 1
                side.run_to(lead + (side.total - lead) * 1.02 * count / ticks, val[r:r + 16, 0:128])

        for c in chunks:
            rest = _dot_nt(weight(G - 1), x_v[pl.ds(c * XC, XC), 512:])
            pace(rest)
            for z in range(XC // 128):
                val = _dot_nt(jnp.concatenate([weight(j) for j in range(G - 1)], 1),
                              x_v[pl.ds(c * XC + 128 * z, 128), :512]) + rest[:, 128 * z:128 * z + 128]
                emit(c * XC // 128 + z, val)
                pace(val)
        side.finish()

    sub = lax.broadcasted_iota(jnp.int32, (8, 128), 0)

    def emit_q(z, val):
        q32[pl.ds(z * D, NA * DH), :] = val[:NA * DH]
        for h in range(H):
            lo, hi = DH * h, DH * (h + 1)
            parts = []
            for r in range(lo // 16 * 16, lo // 16 * 16 + 32, 8):
                part = val[r:r + 8]
                parts.append(jnp.zeros((8, 128), F32) if r + 8 <= lo or r >= hi else
                             jnp.where(sub >= lo - r, part, 0.0) if r < lo else
                             jnp.where(sub < hi - r, part, 0.0) if r + 8 > hi else part)
            qh[h, pl.ds(32 * z, 32), :] = jnp.concatenate(parts, 0).astype(BF16)

    def emit_v(z, val):
        for h in range(0, H, 2):
            r = DH * h
            mid = val[r + 16:r + 24]
            vt[h, pl.ds(32 * z, DV), :] = jnp.concatenate([val[r:r + 16], jnp.where(sub < 4, mid, 1.0)], 0)
            vt[h + 1, pl.ds(32 * z, DV), :] = jnp.concatenate([jnp.where(sub < 4, 1.0, mid), val[r + 24:r + 40]], 0)

    def filter_block(g, z):
        st.add(h_s, (g, pl.ds(z * FB, 128)), ssm_v[pl.ds(128 * g, 128), pl.ds(128 * z, 128)].astype(F32).T, slow)
        yield 40

    def signal_block(g, z):
        cols = pl.ds(128 * g, 128)
        w = shift_v[:, cols].astype(F32)
        base = z % 2 * FB
        stage = kf.at[pl.ds(runtime_zero(zero_s[0]), 2 * FB)]
        stage[pl.ds(base, 8), :] = k_v[pl.ds(128 * z - 16, 16), cols].astype(F32)[8:] if z else jnp.zeros((8, 128), F32)
        stage[pl.ds(base + 8, 128), :] = k_v[pl.ds(128 * z, 128), cols].astype(F32)
        yield 40
        for r in range(0, 128, 32):
            acc = kf[pl.ds(base + 8 + r, 32), :] * w[0:1]
            for t in range(1, KS):
                acc = acc + kf[pl.ds(base + 8 + r - t, 32), :] * w[t:t + 1]
            st.add(u_s, (g, pl.ds(z * FB + r, 32)), acc * v_v[pl.ds(128 * z + r, 32), cols].astype(F32))
            yield 44

    def stores_done():
        st.flush()
        yield 0

    filters = lambda g: [(40, (h_s,), filter_block(g, z)) for z in range(16)]
    signals = lambda i: [(216, (kf, u_s), signal_block(g, z)) for g in range(G) for z in range(8 * i, 8 * i + 8)]
    first = lambda src, dst, g: [(0, (), stores_done())] + [_fft_first(src, dst, st, g, r) for r in range(0, 128, 8)]

    wait(cp_ssm[0])
    items = filters(0)
    for i, item in enumerate(gates(3)):
        items.insert(3 * i, item)
    for g in range(3):
        passes = first(h_s, fh, g)
        for i, item in enumerate(filters(g + 1)):
            passes.insert(1 + i + i * 3 // 4, item)
        items += passes
    project_t(0, (0, 1), emit_q, items)
    wait(cp_k[0], cp_v[0], cp_w[2], cp_ssm[1])
    items = filters(4)
    project_t(0, (2, 3), emit_q, first(h_s, fh, 3) + items[:1]
              + [item for pair in zip(signals(0), weights(1) + items[1:], strict=True) for item in pair])

    kg32, qh32 = kg.bitcast(U32), qh.bitcast(U32)
    kb_row = lambda j, i, d: _low(((j * (NV // 16) + i // 2) * DH + d) * 2 + i % 2)
    qb_row = lambda e, z, d: _top((8 * e + z // 2) * DH + d, z)
    p_row = lambda r, z: 2 * _top(r * NZ + z, z + min(r // 8, 1))

    def spread_keys(h, j, d, nv):
        col = jnp.broadcast_to(k32[h, j, NV - nv:NV, d:d + 1], (nv, 128))
        for i in range(nv // 8):
            work[pl.ds(kb_row(j, (NV - nv) // 8 + i, d), 8), :] = col[8 * i:8 * i + 8]

    def spread_query(h, e, z, d):
        work[pl.ds(qb_row(e, z, d), 8), :] = jnp.broadcast_to(q32[pl.ds(z * D + DH * h + d, 1), :], (8, 128))

    def stage_queries(before, h, z):
        slot = lambda r: pl.ds(_aligned(_top(8 * z + (r & 7), z), 8), 8)
        for i in range(2):
            qw[slot(((DH * before) >> 4) + i), :] = jnp.zeros((8, 128), U32)
        for i in range(2):
            qw[slot(((DH * h) >> 4) + i), :] = qh32[h, pl.ds(16 * z + 8 * i, 8), :]

    def query_tiles(z0, n):
        tiles = [jnp.concatenate([qw[pl.ds(_top(8 * z + r, z), 8), :] for r in range(8)], 0) for z in range(z0, z0 + n)]
        return pltpu.bitcast(jnp.concatenate(tiles, 1), BF16)

    def key_rows(grp, r0, n):
        return pltpu.bitcast(jnp.concatenate([kg32[grp, pl.ds(_low(r), 8), :] for r in range(r0, r0 + n)], 0), BF16)

    def value_tiles(h, k0, n):
        return jnp.concatenate([vt[h, pl.ds(32 * k, DV), :] for k in range(k0, k0 + n)], 1)

    def late_keys():
        for h in range(NA):
            if last_group(h) == G - 1:
                for j in range(NK):
                    k32[h, j, :NV] = pltpu.roll(k32[h, j, :NV], -DH * h % 128, 1)
                    yield 10

    def first_operands():
        for d in range(DH):
            spread_keys(0, 0, d, NV)
            yield 20
        for z in range((NQ - 1) * NZ):
            stage_queries(NA, NA, z)
        for z in range(2 * NZ):
            for d in range(DH):
                spread_query(0, 0, z, d)
            yield 40

    wait(cp_k[1], cp_v[1])
    project_t(1, (0, 1, 2, 3), emit_v,
              [(80, (), late_keys())] + first(h_s, fh, 4) + [(720, (work,), first_operands())] + signals(1)
              + [item for g in range(G) for item in first(u_s, fu, g)])
    wait(cp_tw)

    def vpu_scores(e, a, j, pair, z0, slot, p_out):
        acc = [None, None]
        for d in range(DH):
            keys = jnp.concatenate([work[pl.ds(kb_row(j, 2 * pair + i, d), 8), :] for i in range(2)], 0)
            for i in range(2):
                qrow = work[pl.ds(qb_row(e, a * NZ + z0 + i, d), 8), :]
                term = keys * jnp.concatenate([qrow, qrow], 0)
                acc[i] = acc[i] + term if d else term
            if d == DH - 1:
                for i in range(2):
                    p_out[pl.ds(p_row(slot, z0 + i), 16), :] = jnp.exp2(acc[i]).astype(BF16)
            yield

    def weighted_values(h, t, nv):
        src = (pb0, pb1)[t % 2].bitcast(U32)
        slots = [BK // 16 if nv == NV and r == (BK - NV) // 16 else r for r in range(BK // 16)]
        p = [jnp.concatenate([src[pl.ds(p_row(r, z) // 2, 8), :] for r in slots], 0) for z in range(NZ)]
        return _dot(value_tiles(h, STEPS[t][1] * BK // 128, BK // 128), pltpu.bitcast(jnp.concatenate(p, 1), BF16))

    def head(before, h, after, items, e=0, res=None):
        shared = not items
        side = _SideWork(items, st, runtime_zero(zero_s[0] if isinstance(h, int) else h))
        grp, nxt = key_group(h), jnp.minimum(after, NA - 1)
        nvs = VPU_KEYS[e] if shared else [0] * len(STEPS)
        col = 0 if shared else 256
        pv_span = 52 if shared else 36
        p_outs = [pb.at[pl.ds(side.zero, pb.shape[0] - 64)] for pb in (pb0, pb1)]
        blocks, due = [], []
        for t, (a, j) in enumerate(STEPS):
            if shared:
                blocks += [(a, j, pair, z0, (BK - NV) // 16 + pair, p_outs[t % 2]) for pair in (2, 1) for z0 in (0, 2)]
            due.append(DH * len(blocks))
            if a % 2 == 0 and nvs[NQ * j + NQ - 1] == NV:
                blocks.append((NQ - 1, j, 0, a, BK // 16, p_outs[1]))
                due[-1] += DH // 2
        scores, scored = (None for block in blocks for _ in vpu_scores(e, *block)), 0
        side.run_to(lead)
        if shared and e == 0:
            for z in range(2 * NZ, NQ * NZ):
                for d in range(DH):
                    spread_query(h, 0, z, d)
        acc = {}
        for t, (a, j) in enumerate(STEPS):
            rows = BK - nvs[t]
            s = _dot(key_rows(grp, j * BK // 16, rows // 16), query_tiles(a * NZ, NZ))
            if res is not None:
                side.pin(qw, res[0:8, 0:128])
            if t == 0 or t > len(STEPS) - NQ:
                for z in range(NZ):
                    stage_queries(*((h, after) if t else (before, h)), (a - 1) % NQ * NZ + z)

            def advance(tick, clock, begin=scored):
                nonlocal scored
                frac = clock / (rows + pv_span)
                while scored < begin + (due[t] - begin) * frac - 0.500001:
                    next(scores)
                    scored += 1
                side.run_to(lead + (side.total - lead) * (t + frac) / len(STEPS), tick)

            for r in range(rows // 16):
                for z in range(NZ):
                    p_outs[t % 2][pl.ds(p_row(r, z), 16), :] = jnp.exp2(
                        s[16 * r:16 * r + 16, 128 * z:128 * z + 128]).astype(BF16)
                tick = s[16 * r:16 * r + 8, col:col + 128]
                side.pin(work, tick)
                if shared and r % 3 == 0:
                    jn = (j + 1) % NK
                    spread_keys(h if jn else nxt, jn, a * DH // NQ + r // 3, max(nvs[NQ * jn:NQ * jn + NQ]))
                if shared and r in QUERY_TICKS:
                    i0 = (2 - e) * (len(QUERY_TICKS) * t + QUERY_TICKS.index(r))
                    for i in range(i0, i0 + 2 - e):
                        spread_query(nxt, 1 - e, i // DH, i % DH)
                advance(tick, 16 * (r + 1))
            if t == 0:
                res = weighted_values(before, len(STEPS) - 1, NV * e)
                ot[before, :, pl.ds(S - BQ, BQ)] += res
            else:
                a, j = STEPS[t - 1]
                res = weighted_values(h, t - 1, nvs[t - 1])
                acc[a] = acc[a] + res if j else res
                if t + NQ >= len(STEPS):
                    ot[h, :, pl.ds(a * BQ, BQ)] = acc[a]
            for i, tick in enumerate((res[0:8, 0:128], res[16:24, 0:128], res[8:16, 256:384])):
                side.pin(work, tick)
                advance(tick, rows + pv_span * (i + 1) / 3)
            assert scored == due[t]
        side.finish()
        return res

    def head_pair(i, _):
        h0, h1 = 2 * i, 2 * i + 1
        head(h0, h1, h1 + 1, [], 1, head((h0 - 1) & (H - 1), h0, h1, []))

    def head_with_products(g, _):
        items, back = [], []
        for b in range(16):
            forward, inverse = _fft_middle(fu, fh, work, st, tw_v, g, b)
            items += forward[:1] + back + forward[1:]
            back = [inverse]
        head(NA + g - 1, NA + g, NA + g + 1, items + back)

    lax.fori_loop(0, NM, head_with_products, None)
    head(H - 2, H - 1, 0, [_fft_last(fu, h_s, st, g, r) for g in range(G) for r in range(0, 128, 8)])
    lax.fori_loop(0, NA // 2, head_pair, None)

    def normalize(z):
        cols = pl.ds(_aligned(z * 128, 128), 128)
        parts, lo, hi = [], None, None
        for h in range(0, H, 2):
            even, odd = ot[h, :, cols], ot[h + 1, :, cols]
            denom = jnp.where(sub < 4, odd[0:8], even[16:24])
            lo, hi = (jnp.minimum(lo, denom), jnp.maximum(hi, denom)) if h else (denom, denom)
            inv = 1.0 / denom
            ie, io = inv[4:5], inv[0:1]
            parts += [even[0:16] * ie, jnp.where(sub < 4, even[16:24] * ie, odd[0:8] * io), odd[8:24] * io]
        return jnp.concatenate(parts, 0).T.astype(BF16), jnp.where((lo >= L_LO) & (hi <= L_HI), 0.0, 1.0)

    def mix(z0, o):
        n = o.shape[0]
        rows = pl.ds(_aligned(z0 * 128, 128), n)
        a = _dot(o, wo_v[...])
        gate = jnp.concatenate([gate_s[rows, :]] * G, 1)
        plane = lambda ref: jnp.concatenate([jnp.concatenate(
            [ref[g, pl.ds(_aligned((z0 + z) * FB, 8), 128), :] for z in range(n // 128)], 0) for g in range(G)], 1)
        b = x_v[rows, :].astype(F32) * (plane(h_s) + plane(u_s) * dvec_v[...].astype(F32).reshape(1, D))
        out_v[rows, :] = (gate * a + (1.0 - gate) * b).astype(BF16)

    def out_copy(r0, n, sem):
        return pltpu.make_async_copy(out_v.at[pl.ds(r0, n)], out_hbm.at[pl.ds(r0, n)], osems.at[sem])

    ot[NA - 1, :, pl.ds(S - BQ, BQ)] += weighted_values(NA - 1, len(STEPS) - 1, 0)
    o_first[...], unsafe = normalize(0)
    wait(cp_wo)
    cp_out = [out_copy(sum(OUT[:i]), n, i) for i, n in enumerate(OUT)]
    for i, n in enumerate(OUT):
        z = sum(OUT[:i]) // 128
        if i:
            o, flags = zip(*[normalize(z + e) for e in range(n // 128)])
            unsafe = unsafe + sum(flags)
        mix(z, jnp.concatenate(o, 0) if i else o_first[...])
        cp_out[i].start()
    unsafe = jnp.max(unsafe)
    wait(*cp_out)

    @pl.when(unsafe > 0.0)
    def _():
        def attend(i, _):
            h, z = i // (S // 128), i % (S // 128)
            for r in range(8):
                qw[pl.ds(_top(r, 0), 8), :] = jnp.zeros((8, 128), U32)
            for r in range(2):
                qw[pl.ds(pl.multiple_of(_top((((DH * h) >> 4) + r) & 7, 0), 8), 8), :] = (
                    qh32[h, pl.ds(pl.multiple_of(16 * z + 8 * r, 8), 8), :])
            s = _dot(key_rows(key_group(h), 0, S // 16), query_tiles(0, 1))
            p = jnp.exp2(s - jnp.max(s, axis=0, keepdims=True)).astype(BF16)
            ot[h, :, pl.ds(pl.multiple_of(z * 128, 128), 128)] = _dot(value_tiles(h, 0, S // 128), p)
        lax.fori_loop(0, H * (S // 128), attend, None)
        lax.fori_loop(0, S // 128, lambda z, _: mix(z, normalize(z)[0]), None)
        whole = out_copy(0, S, 0)
        whole.start()
        whole.wait()


@jax.jit
def pallas_gated_mix__mha_block__ssm_conv_h3__prompt_kernel(
    A_x: jax.Array,
    A_wqkv: jax.Array,
    A_wo: jax.Array,
    B_q: jax.Array,
    B_k: jax.Array,
    B_v: jax.Array,
    B_shift_k: jax.Array,
    B_ssm_k: jax.Array,
    B_ssm_D: jax.Array,
    gate_w: jax.Array,
):
    del B_q
    tw = _twiddle_table()
    hbm = pl.BlockSpec(memory_space=pl.ANY)
    vmem = pltpu.VMEM
    out = pl.pallas_call(
        _kernel,
        in_specs=[hbm] * 10,
        out_specs=hbm,
        out_shape=jax.ShapeDtypeStruct((S, D), BF16),
        scratch_shapes=[
            vmem((S, D), BF16), vmem((3, D, D), BF16), vmem((D, D), BF16),
            vmem((S, D), BF16), vmem((S, D), BF16), vmem((D, S), BF16),
            vmem((tw.shape[0], 32, 128), F32), vmem((S, D), BF16),
            vmem((2 * G - 1, 2 * _low(S // 16), 128), BF16),
            vmem((H, S // 4, 128), BF16), vmem((H, S // 4, 128), F32),
            vmem((H, DV, S), F32),
            vmem((G, 16 * FB, 128), F32), vmem((G, 16 * FB, 128), F32),
            vmem((2, G, 16 * FB, 128), F32), vmem((2, G, 16 * FB, 128), F32),
            vmem((NA, NK, NV + 16, 128), F32), vmem((S // 128 * D, 128), F32),
            vmem((WORK_ROWS, 128), F32),
            vmem((4 * NZ * (BK + 16) + 64, 128), BF16),
            vmem((4 * NZ * (BK + 16) + 64, 128), BF16),
            vmem((2 * S + 32, 128), U32), vmem((2 * FB + 16, 128), F32),
            vmem((128, D), BF16), vmem((2, G, D + 64, 128), BF16),
            vmem((S + 32, 128), F32),
            vmem((KS, 1536), BF16), vmem((D,), BF16), vmem((D,), BF16),
            pltpu.SMEM((1,), jnp.int32),
            pltpu.SemaphoreType.DMA((18,)), pltpu.SemaphoreType.DMA((len(OUT),)),
        ],
        compiler_params=pltpu.CompilerParams(vmem_limit_bytes=124 * 2 ** 20),
    )(A_x.reshape(S, D), A_wqkv, A_wo, B_k.reshape(S, D), B_v.reshape(S, D), B_ssm_k, tw,
      B_shift_k.T, B_ssm_D, gate_w)
    return out.reshape(1, S, D)
```
